```python
import os as _os
_os.environ.setdefault('JAX_PLATFORMS', 'cpu')
import jax
import jax.numpy as jnp

def _softmax(x, axis=-1):
    return jax.nn.softmax(x, axis=axis)

def _gelu(x):
    return jax.nn.gelu(x, approximate=True)

def _silu(x):
    return jax.nn.silu(x)

def _sigmoid(x):
    return jax.nn.sigmoid(x)

def _layernorm(x, axis=-1, eps=1e-05):
    m = jnp.mean(x, axis=axis, keepdims=True)
    v = jnp.var(x, axis=axis, keepdims=True)
    return (x - m) / jnp.sqrt(v + eps)

def _scatter_add(tgt, idx, src, axis=0):
    return tgt.at[idx].add(src)

def _segment_sum(src, seg, n):
    return jax.ops.segment_sum(src, seg, n)

class _Rng:

    def __init__(self, key):
        self._k = key

    def _next(self):
        self._k, sub = jax.random.split(self._k)
        return sub

    def normal(self, shape):
        return jax.random.normal(self._next(), shape, dtype=jnp.bfloat16)

    def randint(self, lo, hi, shape):
        return jax.random.randint(self._next(), shape, lo, hi, dtype=jnp.int32)

    def uniform(self, shape, lo=0.0, hi=1.0):
        return jax.random.uniform(self._next(), shape, jnp.bfloat16, lo, hi)

    def permutation(self, n):
        return jax.random.permutation(self._next(), n)
kernel_name = 'adaLN_cond__mha_block_cached__geglu_ffn__prompt'

def setup_inputs():
    _rng = _Rng(jax.random.key(int.from_bytes(__import__("os").urandom(4), "little")))
    _w = lambda a: (lambda t: t.astype(jnp.bfloat16) if jnp.issubdtype(t.dtype, jnp.floating) else t)(jnp.asarray(a))

    def _A_setup():
        B, Sq, D = (1, 2048, 512)
        H, Sk, Dh = (32, 2048, 128)
        return {'x': _w((lambda *s: _rng.normal(s) * 0.05)(B, Sq, D)), 'k_cache': _w((lambda *s: _rng.normal(s) * 3.2)(B, H, Sk, Dh)), 'v_cache': _w((lambda *s: _rng.normal(s) * 0.4)(B, H, Sk, Dh)), 'wq': _w((lambda *s: _rng.normal(s) * 1.6)(D, H * Dh) * D ** (-0.5)), 'wo': _w((lambda *s: _rng.normal(s) * 0.4)(H * Dh, D) * (H * Dh) ** (-0.5))}
    _A_in = _A_setup()

    def _B_setup():
        B, S, D, F = (1, 2048, 512, 1792)
        return {'x': _w((lambda *s: _rng.normal(s) * 0.05)(B, S, D)), 'w_gate': _w((lambda *s: _rng.normal(s) * 0.05)(D, F)), 'w_up': _w((lambda *s: _rng.normal(s) * 0.05)(D, F)), 'w_down': _w((lambda *s: _rng.normal(s) * 0.05)(F, D))}
    _B_in = _B_setup()
    return {'A_x': _A_in['x'], 'A_k_cache': _A_in['k_cache'], 'A_v_cache': _A_in['v_cache'], 'A_wq': _A_in['wq'], 'A_wo': _A_in['wo'], 'B_x': _B_in['x'], 'B_w_gate': _B_in['w_gate'], 'B_w_up': _B_in['w_up'], 'B_w_down': _B_in['w_down'], 'c': _w((lambda *s: _rng.normal(s) * 0.05)(1, 512) * 8.0), 'w_mod': _w((lambda *s: _rng.normal(s) * 0.05)(512, 6 * 512) * 512 ** (-0.5) * 8.0)}

def reference(A_x, A_k_cache, A_v_cache, A_wq, A_wo, B_x, B_w_gate, B_w_up, B_w_down, c, w_mod):

    def _A_ref(x, k_cache, v_cache, wq, wo):
        B, Sq, D = x.shape
        H, Dh = (32, 128)
        q = (lambda x, *d: x.transpose(*d))((x @ wq).reshape(B, Sq, H, Dh), 0, 2, 1, 3)
        scores = jnp.einsum('bhqd,bhkd->bhqk', q, k_cache) * Dh ** (-0.5)
        p = _softmax(scores, axis=-1)
        o = jnp.einsum('bhqk,bhkd->bhqd', p, v_cache)
        return (lambda x, *d: x.transpose(*d))(o, 0, 2, 1, 3).reshape(B, Sq, H * Dh) @ wo

    def _B_ref(x, w_gate, w_up, w_down):
        return _gelu(x @ w_gate) * (x @ w_up) @ w_down
    x = A_x
    mod = (_silu(c) @ w_mod).reshape(c.shape[0], 6, 1, -1)
    sa, ca, ga, sb, cb, gb = (mod[:, 0].copy(), mod[:, 1].copy(), mod[:, 2].copy(), mod[:, 3].copy(), mod[:, 4].copy(), mod[:, 5].copy())
    h = _layernorm(x, axis=-1) * (1 + ca) + sa
    x = x + ga * _A_ref(h, A_k_cache, A_v_cache, A_wq, A_wo)
    h = _layernorm(x, axis=-1) * (1 + cb) + sb
    x = x + gb * _B_ref(h, B_w_gate, B_w_up, B_w_down)
    return x
```

```python
import math
import jax
import jax.numpy as jnp
from jax import lax
from jax.experimental import pallas as pl
from jax.experimental.pallas import tpu as pltpu

S, D, H, DH, SK, F = 2048, 512, 32, 128, 2048, 1792
EPS = 1e-5
LOG2E = 1.4426950408889634
QSCALE = (DH ** -0.5) * LOG2E


def _ln(x):
    m = jnp.mean(x, axis=-1, keepdims=True)
    xc = x - m
    v = jnp.mean(xc * xc, axis=-1, keepdims=True)
    return xc * lax.rsqrt(v + EPS)


def _gelu(x):
    c = math.sqrt(2.0 / math.pi)
    return 0.5 * x * (1.0 + jnp.tanh(c * (x + 0.044715 * (x * x * x))))


def _build(R=256, TM=512, LAG=0, OPLAG=1, XC=4, FLAGS=None, FFN_UNROLL=False):
    NT = S // R
    XR = S // XC
    NTM = S // TM

    def kernel(x_hbm, k_hbm, v_hbm, wq_hbm, wo_hbm, wg_hbm, wu_hbm, wd_hbm, c_hbm, wm_hbm,
               o_hbm,
               x_s, kb, vb, wqb, wob, wg_s, wu_s, wd_s, c_s, wm_s, h_s, acc_s, mod_s, o_s,
               kv_sem, x_sem, w_sem, o_sem):

        def head_copies(h, slot):
            col = pl.ds(pl.multiple_of(h * DH, DH), DH)
            return (
                pltpu.make_async_copy(wq_hbm.at[:, col], wqb.at[slot], kv_sem.at[0, slot]),
                pltpu.make_async_copy(k_hbm.at[0, h], kb.at[slot], kv_sem.at[1, slot]),
                pltpu.make_async_copy(v_hbm.at[0, h], vb.at[slot], kv_sem.at[2, slot]),
                pltpu.make_async_copy(wo_hbm.at[col, :], wob.at[slot], kv_sem.at[3, slot]),
            )

        c_cp = pltpu.make_async_copy(c_hbm, c_s, w_sem.at[0])
        wma_cp = pltpu.make_async_copy(wm_hbm.at[:, 0:2 * D], wm_s.at[:, 0:2 * D], w_sem.at[1])
        wmb_cp = pltpu.make_async_copy(wm_hbm.at[:, 2 * D:6 * D], wm_s.at[:, 2 * D:6 * D], w_sem.at[2])
        wg_cp = pltpu.make_async_copy(wg_hbm, wg_s, w_sem.at[3])
        wu_cp = pltpu.make_async_copy(wu_hbm, wu_s, w_sem.at[4])
        wd_cp = pltpu.make_async_copy(wd_hbm, wd_s, w_sem.at[5])
        x_cps = [pltpu.make_async_copy(x_hbm.at[0, i * XR:(i + 1) * XR, :], x_s.at[i * XR:(i + 1) * XR, :],
                                       x_sem.at[i]) for i in range(XC)]
        c_cp.start()
        wma_cp.start()
        for cp in x_cps:
            cp.start()
        for cp in head_copies(0, 0):
            cp.start()

        c_cp.wait()
        cv = c_s[...].astype(jnp.float32)
        sc = cv * jax.nn.sigmoid(cv)
        sc = jnp.broadcast_to(sc, (16, D)).astype(jnp.bfloat16)
        wma_cp.wait()
        mod_a = jnp.dot(sc, wm_s[:, 0:2 * D], preferred_element_type=jnp.float32)
        sa = mod_a[0:1, 0:D]
        ca1 = 1.0 + mod_a[0:1, D:2 * D]
        mod_s[0:1, 0:D] = sa
        mod_s[1:2, 0:D] = ca1

        for i in range(XC):
            x_cps[i].wait()

            def ln_body(j, carry, i=i):
                r = pl.ds(pl.multiple_of(i * XR + j * 256, 256), 256)
                xv = x_s[r, :].astype(jnp.float32)
                hv = _ln(xv) * mod_s[1:2, 0:D] + mod_s[0:1, 0:D]
                h_s[r, :] = hv.astype(jnp.bfloat16)
                acc_s[r, :] = jnp.zeros((256, D), jnp.float32)
                return carry
            lax.fori_loop(0, XR // 256, ln_body, 0)

        wmb_cp.start()
        wg_cp.start()
        wu_cp.start()
        wd_cp.start()

        def head_body(h, carry):
            slot = lax.rem(h, 2)
            for cp in head_copies(h, slot):
                cp.wait()
            hn = jnp.minimum(h + 1, H - 1)
            for cp in head_copies(hn, 1 - slot):
                cp.start()
            k_ref = kb.at[slot]
            v_ref = vb.at[slot]
            wq_ref = wqb.at[slot]
            wo_ref = wob.at[slot]

            def qk(r):
                q = jnp.dot(h_s[r, :], wq_ref[...], preferred_element_type=jnp.float32)
                q = (q * QSCALE).astype(jnp.bfloat16)
                return lax.dot_general(q, k_ref[...], (((1,), (1,)), ((), ())),
                                       preferred_element_type=jnp.float32)

            def sm(s):
                m = jnp.max(s, axis=-1, keepdims=True)
                p = jnp.exp2(s - m)
                l = jnp.sum(p, axis=-1, keepdims=True)
                return p.astype(jnp.bfloat16), l

            def pv(p, l):
                o = jnp.dot(p, v_ref[...], preferred_element_type=jnp.float32)
                return (o / l).astype(jnp.bfloat16)

            def op(r, o):
                acc_s[r, :] += jnp.dot(o, wo_ref[...], preferred_element_type=jnp.float32)

            rows = [pl.ds(j * R, R) for j in range(NT)]
            ps, os_ = {}, {}
            for t in range(NT + LAG + OPLAG):
                if t < NT:
                    ps[t] = sm(qk(rows[t]))
                j = t - LAG
                if 0 <= j < NT:
                    os_[j] = pv(*ps[j])
                j = t - LAG - OPLAG
                if 0 <= j < NT:
                    op(rows[j], os_[j])
            return carry
        lax.fori_loop(0, H, head_body, 0)
        for cp in head_copies(H - 1, H % 2):
            cp.wait()

        wmb_cp.wait()
        mod_b = jnp.dot(sc, wm_s[:, 2 * D:6 * D], preferred_element_type=jnp.float32)
        mod_s[2:3, 0:D] = mod_b[0:1, 0:D]
        mod_s[3:4, 0:D] = mod_b[0:1, D:2 * D]
        mod_s[4:5, 0:D] = 1.0 + mod_b[0:1, 2 * D:3 * D]
        mod_s[5:6, 0:D] = mod_b[0:1, 3 * D:4 * D]
        wg_cp.wait()
        wu_cp.wait()
        wd_cp.wait()

        def ffn_body(i, carry):
            r = pl.ds(pl.multiple_of(i * TM, TM), TM)
            x1 = x_s[r, :].astype(jnp.float32) + mod_s[2:3, 0:D] * acc_s[r, :]
            h2 = (_ln(x1) * mod_s[4:5, 0:D] + mod_s[3:4, 0:D]).astype(jnp.bfloat16)
            g = jnp.dot(h2, wg_s[...], preferred_element_type=jnp.float32)
            u = jnp.dot(h2, wu_s[...], preferred_element_type=jnp.float32)
            a = (_gelu(g) * u).astype(jnp.bfloat16)
            y = jnp.dot(a, wd_s[...], preferred_element_type=jnp.float32)
            o_s[r, :] = (x1 + mod_s[5:6, 0:D] * y).astype(o_s.dtype)
            pltpu.make_async_copy(o_s.at[r, :], o_hbm.at[0, r, :], o_sem.at[i]).start()
            return carry
        lax.fori_loop(0, NTM, ffn_body, 0, unroll=FFN_UNROLL)
        for i in range(NTM):
            r = pl.ds(i * TM, TM)
            pltpu.make_async_copy(o_s.at[r, :], o_hbm.at[0, r, :], o_sem.at[i]).wait()

    @jax.jit
    def fn(A_x, A_k_cache, A_v_cache, A_wq, A_wo, B_x, B_w_gate, B_w_up, B_w_down, c, w_mod):
        any_spec = pl.BlockSpec(memory_space=pl.ANY)
        bf = jnp.bfloat16
        return pl.pallas_call(
            kernel,
            in_specs=[any_spec] * 10,
            out_specs=any_spec,
            out_shape=jax.ShapeDtypeStruct((1, S, D), A_x.dtype),
            scratch_shapes=[
                pltpu.VMEM((S, D), bf),
                pltpu.VMEM((2, SK, DH), bf),
                pltpu.VMEM((2, SK, DH), bf),
                pltpu.VMEM((2, D, DH), bf),
                pltpu.VMEM((2, DH, D), bf),
                pltpu.VMEM((D, F), bf),
                pltpu.VMEM((D, F), bf),
                pltpu.VMEM((F, D), bf),
                pltpu.VMEM((1, D), bf),
                pltpu.VMEM((D, 6 * D), bf),
                pltpu.VMEM((S, D), bf),
                pltpu.VMEM((S, D), jnp.float32),
                pltpu.VMEM((8, D), jnp.float32),
                pltpu.VMEM((S, D), bf),
                pltpu.SemaphoreType.DMA((4, 2)),
                pltpu.SemaphoreType.DMA((XC,)),
                pltpu.SemaphoreType.DMA((6,)),
                pltpu.SemaphoreType.DMA((NTM,)),
            ],
            compiler_params=pltpu.CompilerParams(
                vmem_limit_bytes=100 * 1024 * 1024,
                flags=FLAGS,
            ),
        )(A_x, A_k_cache, A_v_cache, A_wq, A_wo, B_w_gate, B_w_up, B_w_down, c, w_mod)
    return fn


_impl = _build()


@jax.jit
def pallas_adaLN_cond__mha_block_cached__geglu_ffn__prompt_kernel(
    A_x, A_k_cache, A_v_cache, A_wq, A_wo, B_x, B_w_gate, B_w_up, B_w_down, c, w_mod,
):
    return _impl(A_x, A_k_cache, A_v_cache, A_wq, A_wo, B_x, B_w_gate, B_w_up, B_w_down, c, w_mod)
```

```python
import math
import jax
import jax.numpy as jnp
from jax import lax
from jax.experimental import pallas as pl
from jax.experimental.pallas import tpu as pltpu

S, D, H, DH, SK, F = 2048, 512, 32, 128, 2048, 1792
EPS = 1e-5
LOG2E = 1.4426950408889634
QSCALE = (DH ** -0.5) * LOG2E


def _ln(x):
    m = jnp.mean(x, axis=-1, keepdims=True)
    xc = x - m
    v = jnp.mean(xc * xc, axis=-1, keepdims=True)
    return xc * lax.rsqrt(v + EPS)


def _gelu(x):
    c = math.sqrt(2.0 / math.pi)
    return 0.5 * x * (1.0 + jnp.tanh(c * (x + 0.044715 * (x * x * x))))


def _build(R=256, TM=512, OPLAG=2, ORDER='kqov', CUT=3, XC=8, FLAGS=None, SCOPES=False, RS=(256,) * 7 + (192, 64)):
    RS = RS or [R] * (S // R)
    assert sum(RS) == S
    R = max(RS)
    NT = len(RS)
    R0 = [sum(RS[:j]) for j in range(NT)]
    seq = []
    for t in range(0, 2 * NT):
        for st in ORDER:
            off = {'k': 0, 'q': 1, 'o': -OPLAG, 'v': 0}[st]
            seq.append((st, t + off))
    PROG = seq[CUT:CUT + len(ORDER) * NT]
    produced = set()
    carried = set()
    for st, n in PROG:
        need = {'q': [], 'k': [('Q', n)], 'v': [('S', n), ('M', n)], 'o': [('O', n)]}[st]
        for d in need:
            if d not in produced:
                carried.add(d)
        outs = {'q': [('Q', n)], 'k': [('S', n), ('M', n)], 'v': [('O', n)], 'o': []}[st]
        produced.update(outs)
    NCO = max(1, sum(1 for k, n in carried if k == 'O'))
    NCQ = max(1, sum(1 for k, n in carried if k == 'Q'))
    NCS = max(1, sum(1 for k, n in carried if k == 'S'))
    KB = 3 if any(st == 'k' and n >= NT for st, n in PROG) else 2
    KPF = KB - 1
    XR = S // XC
    NTM = S // TM
    import contextlib
    scope = (lambda n: jax.named_scope(n)) if SCOPES else (lambda n: contextlib.nullcontext())

    def kernel(x_hbm, k_hbm, v_hbm, wq_hbm, wo_hbm, wg_hbm, wu_hbm, wd_hbm, c_hbm, wm_hbm,
               o_hbm,
               x_s, kb, vb, wq_s, wo_s, wg_s, wu_s, wd_s, c_s, wm_s, h_s, acc_s, mod_s, o_s,
               q0_s, oc_s, s_s, m_s,
               kv_sem, x_sem, w_sem, o_sem):

        def k_copy(hh, j):
            slot = lax.rem(j, KB) if not isinstance(j, int) else j % KB
            return pltpu.make_async_copy(k_hbm.at[0, hh], kb.at[slot], kv_sem.at[slot])

        def v_copy(hh, j):
            slot = lax.rem(j, 2) if not isinstance(j, int) else j % 2
            return pltpu.make_async_copy(v_hbm.at[0, hh], vb.at[slot], kv_sem.at[4 + slot])

        def wq_copy(h_src, j_dst):
            col = pl.ds(pl.multiple_of(h_src * DH, DH), DH)
            return pltpu.make_async_copy(wq_hbm.at[:, col], wq_s.at[j_dst], w_sem.at[6])

        def wo_copy(h_src, j_dst):
            col = pl.ds(pl.multiple_of(h_src * DH, DH), DH)
            return pltpu.make_async_copy(wo_hbm.at[col, :], wo_s.at[j_dst], w_sem.at[7])

        c_cp = pltpu.make_async_copy(c_hbm, c_s, w_sem.at[0])
        wma_cp = pltpu.make_async_copy(wm_hbm.at[:, 0:2 * D], wm_s.at[:, 0:2 * D], w_sem.at[1])
        wmb_cp = pltpu.make_async_copy(wm_hbm.at[:, 2 * D:6 * D], wm_s.at[:, 2 * D:6 * D], w_sem.at[2])
        wg_cp = pltpu.make_async_copy(wg_hbm, wg_s, w_sem.at[3])
        wu_cp = pltpu.make_async_copy(wu_hbm, wu_s, w_sem.at[4])
        wd_cp = pltpu.make_async_copy(wd_hbm, wd_s, w_sem.at[5])
        x_cps = [pltpu.make_async_copy(x_hbm.at[0, i * XR:(i + 1) * XR, :], x_s.at[i * XR:(i + 1) * XR, :],
                                       x_sem.at[i]) for i in range(XC)]
        c_cp.start()
        wma_cp.start()
        for cp in x_cps:
            cp.start()
        wq_copy(0, 0).start()
        for j in range(KPF):
            k_copy(j, j).start()
        v_copy(0, 0).start()

        wo_s[0] = jnp.zeros((DH, D), jnp.bfloat16)
        oc_s[...] = jnp.zeros(oc_s.shape, jnp.bfloat16)

        with scope('wait_c'):
            c_cp.wait()
        cv = c_s[...].astype(jnp.float32)
        sc = cv * jax.nn.sigmoid(cv)
        sc = jnp.broadcast_to(sc, (16, D)).astype(jnp.bfloat16)
        with scope('wait_wma'):
            wma_cp.wait()
        mod_a = jnp.dot(sc, wm_s[:, 0:2 * D], preferred_element_type=jnp.float32)
        mod_s[0:1, 0:D] = mod_a[0:1, 0:D]
        mod_s[1:2, 0:D] = 1.0 + mod_a[0:1, D:2 * D]

        def ln_body(j, carry):
            pltpu.make_async_copy(x_hbm.at[0, pl.ds(0, XR), :], x_s.at[pl.ds(0, XR), :], x_sem.at[j]).wait()
            r = pl.ds(pl.multiple_of(j * XR, XR), XR)
            xv = x_s[r, :].astype(jnp.float32)
            hv = _ln(xv) * mod_s[1:2, 0:D] + mod_s[0:1, 0:D]
            h_s[r, :] = hv.astype(jnp.bfloat16)
            acc_s[r, :] = jnp.zeros((XR, D), jnp.float32)
            return carry
        with scope('ln'):
            lax.fori_loop(0, XC, ln_body, 0)

        wq_copy(0, 0).wait()
        wq_copy(1, 1).start()
        wo_copy(0, 1).start()
        wmb_cp.start()
        wg_cp.start()
        wu_cp.start()
        wd_cp.start()

        def qp(r, wq_ref):
            q = jnp.dot(h_s[r, :], wq_ref[...], preferred_element_type=jnp.float32)
            return (q * QSCALE).astype(jnp.bfloat16)

        def op(r, o, wo_ref):
            acc_s[r, :] += jnp.dot(o, wo_ref[...], preferred_element_type=jnp.float32)

        rows = [pl.ds(R0[j], RS[j]) for j in range(NT)]
        for kind, n in sorted(carried):
            if kind == 'Q':
                q0_s[n % NCQ, 0:RS[n]] = qp(rows[n], wq_s.at[0])
        if KB == 3:
            k_copy(0, 0).wait()
        for kind, n in sorted(carried):
            if kind == 'S':
                s0 = lax.dot_general(qp(rows[n], wq_s.at[0]), kb[0], (((1,), (1,)), ((), ())),
                                     preferred_element_type=jnp.float32)
                s_s[n % NCS, 0:RS[n]] = s0
                m_s[n % NCS, 0:RS[n]] = jnp.broadcast_to(jnp.max(s0, axis=-1, keepdims=True), (RS[n], 128))

        def head_body(h, carry):
            k_copy(h, h + KPF - 1).wait()
            v_copy(h, h).wait()
            wq_copy(h, h + 1).wait()
            wo_copy(h, h + 1).wait()
            hn = jnp.minimum(h + 1, H - 1)
            k_copy(jnp.minimum(h + KPF, H - 1), h + KPF).start()
            v_copy(hn, h + 1).start()
            wq_copy(jnp.minimum(h + 2, H - 1), h + 2).start()
            wo_copy(hn, h + 2).start()
            v_ref = vb.at[lax.rem(h, 2)]

            def kref(n):
                return kb.at[lax.rem(h + n // NT, KB)] if n // NT else kb.at[lax.rem(h, KB)]

            vals = {}

            def get(kind, n):
                if (kind, n) in vals:
                    return vals[(kind, n)]
                assert n < 0 or kind in ('S', 'M', 'Q'), (kind, n)
                sz = RS[n % NT]
                if kind == 'O':
                    return oc_s[n % NCO, 0:sz]
                if kind == 'Q':
                    return q0_s[n % NCQ, 0:sz]
                if kind == 'S':
                    return s_s[n % NCS, 0:sz]
                if kind == 'M':
                    return m_s[n % NCS, 0:sz]

            def put(kind, n, val):
                vals[(kind, n)] = val
                if (kind, n - NT) in carried:
                    sz = RS[n % NT]
                    if kind == 'O':
                        oc_s[(n - NT) % NCO, 0:sz] = val
                    elif kind == 'Q':
                        q0_s[(n - NT) % NCQ, 0:sz] = val
                    elif kind == 'S':
                        s_s[(n - NT) % NCS, 0:sz] = val
                    elif kind == 'M':
                        m_s[(n - NT) % NCS, 0:sz] = jnp.broadcast_to(val, (sz, 128))

            for st, n in PROG:
                hd = n // NT
                r = rows[n % NT]
                if st == 'q':
                    put('Q', n, qp(r, wq_s.at[h + hd]))
                elif st == 'k':
                    s = lax.dot_general(get('Q', n), kref(n)[...], (((1,), (1,)), ((), ())),
                                        preferred_element_type=jnp.float32)
                    put('S', n, s)
                    put('M', n, jnp.max(s, axis=-1, keepdims=True))
                elif st == 'v':
                    s = get('S', n)
                    m = get('M', n)
                    if m.shape[1] != 1:
                        m = jnp.concatenate([m] * (SK // 128), axis=1)
                    p = jnp.exp2(s - m)
                    l = jnp.sum(p, axis=-1, keepdims=True)
                    o = jnp.dot(p.astype(jnp.bfloat16), v_ref[...], preferred_element_type=jnp.float32)
                    put('O', n, (o / l).astype(jnp.bfloat16))
                elif st == 'o':
                    op(r, get('O', n), wo_s.at[h + 1 + hd])
            return carry
        with scope('heads'):
            lax.fori_loop(0, H, head_body, 0)
        k_copy(0, H + KPF - 1).wait()
        v_copy(0, H).wait()
        wq_copy(0, H + 1).wait()
        wo_copy(0, H + 1).wait()
        for kind, n in sorted(carried):
            if kind == 'O':
                op(rows[n % NT], oc_s[n % NCO, 0:RS[n % NT]], wo_s.at[H])

        wmb_cp.wait()
        mod_b = jnp.dot(sc, wm_s[:, 2 * D:6 * D], preferred_element_type=jnp.float32)
        mod_s[2:3, 0:D] = mod_b[0:1, 0:D]
        mod_s[3:4, 0:D] = mod_b[0:1, D:2 * D]
        mod_s[4:5, 0:D] = 1.0 + mod_b[0:1, 2 * D:3 * D]
        mod_s[5:6, 0:D] = mod_b[0:1, 3 * D:4 * D]
        wg_cp.wait()
        wu_cp.wait()
        wd_cp.wait()

        def ffn_body(i, carry):
            r = pl.ds(pl.multiple_of(i * TM, TM), TM)
            x1 = x_s[r, :].astype(jnp.float32) + mod_s[2:3, 0:D] * acc_s[r, :]
            h2 = (_ln(x1) * mod_s[4:5, 0:D] + mod_s[3:4, 0:D]).astype(jnp.bfloat16)
            g = jnp.dot(h2, wg_s[...], preferred_element_type=jnp.float32)
            u = jnp.dot(h2, wu_s[...], preferred_element_type=jnp.float32)
            a = (_gelu(g) * u).astype(jnp.bfloat16)
            y = jnp.dot(a, wd_s[...], preferred_element_type=jnp.float32)
            o_s[r, :] = (x1 + mod_s[5:6, 0:D] * y).astype(o_s.dtype)
            pltpu.make_async_copy(o_s.at[r, :], o_hbm.at[0, r, :], o_sem.at[i]).start()
            return carry
        with scope('ffn'):
            lax.fori_loop(0, NTM, ffn_body, 0)
        with scope('wait_out'):
            for i in range(NTM):
                r = pl.ds(i * TM, TM)
                pltpu.make_async_copy(o_s.at[r, :], o_hbm.at[0, r, :], o_sem.at[i]).wait()

    @jax.jit
    def fn(A_x, A_k_cache, A_v_cache, A_wq, A_wo, B_x, B_w_gate, B_w_up, B_w_down, c, w_mod):
        any_spec = pl.BlockSpec(memory_space=pl.ANY)
        bf = jnp.bfloat16
        return pl.pallas_call(
            kernel,
            in_specs=[any_spec] * 10,
            out_specs=any_spec,
            out_shape=jax.ShapeDtypeStruct((1, S, D), A_x.dtype),
            scratch_shapes=[
                pltpu.VMEM((S, D), bf),
                pltpu.VMEM((KB, SK, DH), bf),
                pltpu.VMEM((2, SK, DH), bf),
                pltpu.VMEM((H + 2, D, DH), bf),
                pltpu.VMEM((H + 2, DH, D), bf),
                pltpu.VMEM((D, F), bf),
                pltpu.VMEM((D, F), bf),
                pltpu.VMEM((F, D), bf),
                pltpu.VMEM((1, D), bf),
                pltpu.VMEM((D, 6 * D), bf),
                pltpu.VMEM((S, D), bf),
                pltpu.VMEM((S, D), jnp.float32),
                pltpu.VMEM((8, D), jnp.float32),
                pltpu.VMEM((S, D), bf),
                pltpu.VMEM((NCQ, R, DH), bf),
                pltpu.VMEM((NCO, R, DH), bf),
                pltpu.VMEM((NCS, R, SK), jnp.float32),
                pltpu.VMEM((NCS, R, 128), jnp.float32),
                pltpu.SemaphoreType.DMA((6,)),
                pltpu.SemaphoreType.DMA((XC,)),
                pltpu.SemaphoreType.DMA((8,)),
                pltpu.SemaphoreType.DMA((NTM,)),
            ],
            compiler_params=pltpu.CompilerParams(
                vmem_limit_bytes=100 * 1024 * 1024,
                flags=FLAGS,
            ),
        )(A_x, A_k_cache, A_v_cache, A_wq, A_wo, B_w_gate, B_w_up, B_w_down, c, w_mod)
    return fn


_impl = _build()


@jax.jit
def pallas_adaLN_cond__mha_block_cached__geglu_ffn__prompt_kernel(
    A_x, A_k_cache, A_v_cache, A_wq, A_wo, B_x, B_w_gate, B_w_up, B_w_down, c, w_mod,
):
    return _impl(A_x, A_k_cache, A_v_cache, A_wq, A_wo, B_x, B_w_gate, B_w_up, B_w_down, c, w_mod)
```

```python
import math
import jax
import jax.numpy as jnp
from jax import lax
from jax.experimental import pallas as pl
from jax.experimental.pallas import tpu as pltpu

S, D, H, DH, SK, F = 2048, 512, 32, 128, 2048, 1792
EPS = 1e-5
LOG2E = 1.4426950408889634
QSCALE = (DH ** -0.5) * LOG2E


def _ln(x):
    m = jnp.mean(x, axis=-1, keepdims=True)
    xc = x - m
    v = jnp.mean(xc * xc, axis=-1, keepdims=True)
    return xc * lax.rsqrt(v + EPS)


def _recip(l):
    r = pl.reciprocal(l, approx=True)
    r = r + r * (1.0 - l * r)
    return r


def _gelu(x):
    c = math.sqrt(2.0 / math.pi)
    return 0.5 * x * (1.0 + jnp.tanh(c * (x + 0.044715 * (x * x * x))))


def _build(R=256, TM=512, OPLAG=2, ORDER='kqov', CUT=0, XC=8, FLAGS=None, SCOPES=False, RS=None, BC=1, W0=1, W1=2, W2=1, NOFFN=False):
    RS = RS or [R] * (S // R)
    assert sum(RS) == S
    R = max(RS)
    NT = len(RS)
    R0 = [sum(RS[:j]) for j in range(NT)]
    seq = []
    for t in range(0, 2 * NT):
        for st in ORDER:
            off = {'k': 0, 'q': 1, 'o': -OPLAG, 'v': 0}[st]
            seq.append((st, t + off))
    PROG = seq[CUT:CUT + len(ORDER) * NT]
    produced = set()
    carried = set()
    for st, n in PROG:
        need = {'q': [], 'k': [('Q', n)], 'v': [('S', n), ('M', n)], 'o': [('O', n)]}[st]
        for d in need:
            if d not in produced:
                carried.add(d)
        outs = {'q': [('Q', n)], 'k': [('S', n), ('M', n)], 'v': [('O', n)], 'o': []}[st]
        produced.update(outs)
    NCO = max(1, sum(1 for k, n in carried if k == 'O'))
    NCQ = max(1, sum(1 for k, n in carried if k == 'Q'))
    NCS = max(1, sum(1 for k, n in carried if k == 'S'))
    KB = 3 if any(st == 'k' and n >= NT for st, n in PROG) else 2
    KPF = KB - 1
    XR = S // XC
    NTM = S // TM
    import contextlib
    scope = (lambda n: jax.named_scope(n)) if SCOPES else (lambda n: contextlib.nullcontext())

    def kernel(x_hbm, k_hbm, v_hbm, wq_hbm, wo_hbm, wg_hbm, wu_hbm, wd_hbm, c_hbm, wm_hbm,
               o_hbm,
               x_s, kb, vb, wq_s, wo_s, wg_s, wu_s, wd_s, c_s, wm_s, h_s, acc_s, mod_s, o_s,
               q0_s, oc_s, s_s, m_s,
               kv_sem, x_sem, w_sem, o_sem):

        def k_copy(hh, j):
            slot = lax.rem(j, KB) if not isinstance(j, int) else j % KB
            return pltpu.make_async_copy(k_hbm.at[0, hh], kb.at[slot], kv_sem.at[slot])

        def v_copy(hh, j):
            slot = lax.rem(j, 2) if not isinstance(j, int) else j % 2
            return pltpu.make_async_copy(v_hbm.at[0, hh], vb.at[slot], kv_sem.at[4 + slot])

        def wq_copy(h_src, j_dst):
            col = pl.ds(pl.multiple_of(h_src * DH, DH), DH)
            return pltpu.make_async_copy(wq_hbm.at[:, col], wq_s.at[j_dst], w_sem.at[6])

        def wo_copy(h_src, j_dst):
            col = pl.ds(pl.multiple_of(h_src * DH, DH), DH)
            return [pltpu.make_async_copy(wo_hbm.at[col, b * 128:(b + 1) * 128], wo_s.at[j_dst, b], w_sem.at[7])
                    for b in range(D // 128)]

        c_cp = pltpu.make_async_copy(c_hbm, c_s, w_sem.at[0])
        wma_cp = pltpu.make_async_copy(wm_hbm.at[:, 0:2 * D], wm_s.at[:, 0:2 * D], w_sem.at[1])
        wmb_cp = pltpu.make_async_copy(wm_hbm.at[:, 2 * D:6 * D], wm_s.at[:, 2 * D:6 * D], w_sem.at[2])
        wg_cp = pltpu.make_async_copy(wg_hbm, wg_s, w_sem.at[3])
        wu_cp = pltpu.make_async_copy(wu_hbm, wu_s, w_sem.at[4])
        wd_cp = pltpu.make_async_copy(wd_hbm, wd_s, w_sem.at[5])
        x_cps = [pltpu.make_async_copy(x_hbm.at[0, i * XR:(i + 1) * XR, :], x_s.at[i * XR:(i + 1) * XR, :],
                                       x_sem.at[i]) for i in range(XC)]
        def start_item(it):
            kind, j = it
            if kind == 'x':
                x_cps[j].start()
            elif kind == 'wq':
                wq_copy(j, j).start()
            elif kind == 'k':
                k_copy(j, j).start()
            elif kind == 'v':
                v_copy(j, j).start()
            elif kind == 'wo':
                for cp in wo_copy(j, j + 1):
                    cp.start()

        items = [('x', j) for j in range(XC)] + [('wq', 0), ('k', 0), ('v', 0), ('wq', 1), ('wo', 0)]
        if KB == 3:
            items.append(('k', 1))
        pos = 0
        c_cp.start()
        wma_cp.start()
        for it in items[:W0]:
            start_item(it)
        pos = W0

        wo_s[0] = jnp.zeros((D // 128, DH, 128), jnp.bfloat16)
        oc_s[...] = jnp.zeros(oc_s.shape, jnp.bfloat16)
        acc_s[...] = jnp.zeros(acc_s.shape, jnp.float32)

        with scope('wait_c'):
            c_cp.wait()
        cv = c_s[...].astype(jnp.float32)
        sc = cv * jax.nn.sigmoid(cv)
        sc = jnp.broadcast_to(sc, (16, D)).astype(jnp.bfloat16)
        with scope('wait_wma'):
            wma_cp.wait()
        for it in items[pos:pos + W1]:
            start_item(it)
        pos += W1
        mod_a = jnp.dot(sc, wm_s[:, 0:2 * D], preferred_element_type=jnp.float32)
        mod_s[0:1, 0:D] = mod_a[0:1, 0:D]
        mod_s[1:2, 0:D] = 1.0 + mod_a[0:1, D:2 * D]

        with scope('ln'):
            for j in range(XC):
                x_cps[j].wait()
                nst = W2 if j < XC - 1 else len(items)
                for it in items[pos:pos + nst]:
                    start_item(it)
                pos += nst
                r = pl.ds(j * XR, XR)
                xv = x_s[r, :].astype(jnp.float32)
                hv = _ln(xv) * mod_s[1:2, 0:D] + mod_s[0:1, 0:D]
                hb = hv.astype(jnp.bfloat16)
                r2 = pl.ds(j * (XR // 2), XR // 2)
                for b in range(D // 128):
                    h_s[b, r2, :] = pltpu.bitcast(hb[:, b * 128:(b + 1) * 128], jnp.uint32)

        with scope('wait_wq'):
            wq_copy(0, 0).wait()
        wmb_cp.start()
        wg_cp.start()
        wu_cp.start()
        wd_cp.start()

        def ldw(ref):
            if not BC:
                return ref[...]
            return pltpu.bitcast(ref.bitcast(jnp.uint32)[...], jnp.bfloat16)

        def qp(j, wq_ref):
            r2 = pl.ds(R0[j] // 2, RS[j] // 2)
            hh = jnp.concatenate([pltpu.bitcast(h_s[b, r2, :], jnp.bfloat16) for b in range(D // 128)], axis=1)
            q = jnp.dot(hh, ldw(wq_ref), preferred_element_type=jnp.float32)
            return (q * QSCALE).astype(jnp.bfloat16)

        def op(r, o, wo_ref):
            w = jnp.concatenate([ldw(wo_ref.at[b]) for b in range(D // 128)], axis=1)
            acc_s[r, :] += jnp.dot(o, w, preferred_element_type=jnp.float32)

        rows = [pl.ds(R0[j], RS[j]) for j in range(NT)]
        for kind, n in sorted(carried):
            if kind == 'Q':
                q0_s[n % NCQ, 0:RS[n]] = qp(n, wq_s.at[0])
        if KB == 3:
            k_copy(0, 0).wait()
        for kind, n in sorted(carried):
            if kind == 'S':
                s0 = lax.dot_general(qp(n, wq_s.at[0]), ldw(kb.at[0]), (((1,), (1,)), ((), ())),
                                     preferred_element_type=jnp.float32)
                s_s[n % NCS, 0:RS[n]] = s0
                m_s[n % NCS, 0:RS[n]] = jnp.broadcast_to(jnp.max(s0, axis=-1, keepdims=True), (RS[n], 128))

        def head_body(h, carry):
            k_copy(h, h + KPF - 1).wait()
            v_copy(h, h).wait()
            wq_copy(h, h + 1).wait()
            for cp in wo_copy(h, h + 1):
                cp.wait()
            hn = jnp.minimum(h + 1, H - 1)
            k_copy(jnp.minimum(h + KPF, H - 1), h + KPF).start()
            v_copy(hn, h + 1).start()
            wq_copy(jnp.minimum(h + 2, H - 1), h + 2).start()
            for cp in wo_copy(hn, h + 2):
                cp.start()
            v_ref = vb.at[lax.rem(h, 2)]

            def kref(n):
                return kb.at[lax.rem(h + n // NT, KB)] if n // NT else kb.at[lax.rem(h, KB)]

            vals = {}

            def get(kind, n):
                if (kind, n) in vals:
                    return vals[(kind, n)]
                assert n < 0 or kind in ('S', 'M', 'Q'), (kind, n)
                sz = RS[n % NT]
                if kind == 'O':
                    return oc_s[n % NCO, 0:sz]
                if kind == 'Q':
                    return q0_s[n % NCQ, 0:sz]
                if kind == 'S':
                    return s_s[n % NCS, 0:sz]
                if kind == 'M':
                    return m_s[n % NCS, 0:sz]

            def put(kind, n, val):
                vals[(kind, n)] = val
                if (kind, n - NT) in carried:
                    sz = RS[n % NT]
                    if kind == 'O':
                        oc_s[(n - NT) % NCO, 0:sz] = val
                    elif kind == 'Q':
                        q0_s[(n - NT) % NCQ, 0:sz] = val
                    elif kind == 'S':
                        s_s[(n - NT) % NCS, 0:sz] = val
                    elif kind == 'M':
                        m_s[(n - NT) % NCS, 0:sz] = jnp.broadcast_to(val, (sz, 128))

            for st, n in PROG:
                hd = n // NT
                r = rows[n % NT]
                if st == 'q':
                    put('Q', n, qp(n % NT, wq_s.at[h + hd]))
                elif st == 'k':
                    s = lax.dot_general(get('Q', n), ldw(kref(n)), (((1,), (1,)), ((), ())),
                                        preferred_element_type=jnp.float32)
                    put('S', n, s)
                    put('M', n, jnp.max(s, axis=-1, keepdims=True))
                elif st == 'v':
                    s = get('S', n)
                    m = get('M', n)
                    if m.shape[1] != 1:
                        m = jnp.concatenate([m] * (SK // 128), axis=1)
                    p = jnp.exp2(s - m)
                    l = jnp.sum(p, axis=-1, keepdims=True)
                    o = jnp.dot(p.astype(jnp.bfloat16), ldw(v_ref), preferred_element_type=jnp.float32)
                    put('O', n, (o * _recip(l)).astype(jnp.bfloat16))
                elif st == 'o':
                    op(r, get('O', n), wo_s.at[h + 1 + hd])
            return carry
        with scope('heads'):
            lax.fori_loop(0, H, head_body, 0)
        k_copy(0, H + KPF - 1).wait()
        v_copy(0, H).wait()
        wq_copy(0, H + 1).wait()
        for cp in wo_copy(0, H + 1):
            cp.wait()
        for kind, n in sorted(carried):
            if kind == 'O':
                op(rows[n % NT], oc_s[n % NCO, 0:RS[n % NT]], wo_s.at[H])

        if NOFFN:
            wmb_cp.wait(); wg_cp.wait(); wu_cp.wait(); wd_cp.wait()
            o_s[...] = acc_s[...].astype(o_s.dtype)
            cp = pltpu.make_async_copy(o_s, o_hbm.at[0], o_sem.at[0])
            cp.start(); cp.wait()
        else:
            wmb_cp.wait()
            mod_b = jnp.dot(sc, wm_s[:, 2 * D:6 * D], preferred_element_type=jnp.float32)
            mod_s[2:3, 0:D] = mod_b[0:1, 0:D]
            mod_s[3:4, 0:D] = mod_b[0:1, D:2 * D]
            mod_s[4:5, 0:D] = 1.0 + mod_b[0:1, 2 * D:3 * D]
            mod_s[5:6, 0:D] = mod_b[0:1, 3 * D:4 * D]
            wg_cp.wait()
            wu_cp.wait()
            wd_cp.wait()

            def h2_tile(i):
                r = pl.ds(pl.multiple_of(i * TM, TM), TM)
                x1 = x_s[r, :].astype(jnp.float32) + mod_s[2:3, 0:D] * acc_s[r, :]
                hb = (_ln(x1) * mod_s[4:5, 0:D] + mod_s[3:4, 0:D]).astype(jnp.bfloat16)
                r2 = pl.ds(pl.multiple_of(i * (TM // 2), TM // 2), TM // 2)
                for b in range(D // 128):
                    h_s[b, r2, :] = pltpu.bitcast(hb[:, b * 128:(b + 1) * 128], jnp.uint32)

            h2_tile(0)

            def ffn_body(i, carry):
                r = pl.ds(pl.multiple_of(i * TM, TM), TM)
                r2 = pl.ds(pl.multiple_of(i * (TM // 2), TM // 2), TM // 2)
                h2 = jnp.concatenate([pltpu.bitcast(h_s[b, r2, :], jnp.bfloat16) for b in range(D // 128)], axis=1)
                g = jnp.dot(h2, wg_s[...], preferred_element_type=jnp.float32)
                u = jnp.dot(h2, wu_s[...], preferred_element_type=jnp.float32)
                a = (_gelu(g) * u).astype(jnp.bfloat16)
                h2_tile(lax.rem(i + 1, NTM))
                y = jnp.dot(a, wd_s[...], preferred_element_type=jnp.float32)
                x1 = x_s[r, :].astype(jnp.float32) + mod_s[2:3, 0:D] * acc_s[r, :]
                o_s[r, :] = (x1 + mod_s[5:6, 0:D] * y).astype(o_s.dtype)
                pltpu.make_async_copy(o_s.at[r, :], o_hbm.at[0, r, :], o_sem.at[i]).start()
                return carry
            with scope('ffn'):
                lax.fori_loop(0, NTM, ffn_body, 0)
            with scope('wait_out'):
                for i in range(NTM):
                    r = pl.ds(i * TM, TM)
                    pltpu.make_async_copy(o_s.at[r, :], o_hbm.at[0, r, :], o_sem.at[i]).wait()

    @jax.jit
    def fn(A_x, A_k_cache, A_v_cache, A_wq, A_wo, B_x, B_w_gate, B_w_up, B_w_down, c, w_mod):
        any_spec = pl.BlockSpec(memory_space=pl.ANY)
        bf = jnp.bfloat16
        return pl.pallas_call(
            kernel,
            in_specs=[any_spec] * 10,
            out_specs=any_spec,
            out_shape=jax.ShapeDtypeStruct((1, S, D), A_x.dtype),
            scratch_shapes=[
                pltpu.VMEM((S, D), bf),
                pltpu.VMEM((KB, SK, DH), bf),
                pltpu.VMEM((2, SK, DH), bf),
                pltpu.VMEM((H + 2, D, DH), bf),
                pltpu.VMEM((H + 2, D // 128, DH, 128), bf),
                pltpu.VMEM((D, F), bf),
                pltpu.VMEM((D, F), bf),
                pltpu.VMEM((F, D), bf),
                pltpu.VMEM((1, D), bf),
                pltpu.VMEM((D, 6 * D), bf),
                pltpu.VMEM((D // 128, S // 2, 128), jnp.uint32),
                pltpu.VMEM((S, D), jnp.float32),
                pltpu.VMEM((8, D), jnp.float32),
                pltpu.VMEM((S, D), bf),
                pltpu.VMEM((NCQ, R, DH), bf),
                pltpu.VMEM((NCO, R, DH), bf),
                pltpu.VMEM((NCS, R, SK), jnp.float32),
                pltpu.VMEM((NCS, R, 128), jnp.float32),
                pltpu.SemaphoreType.DMA((6,)),
                pltpu.SemaphoreType.DMA((XC,)),
                pltpu.SemaphoreType.DMA((8,)),
                pltpu.SemaphoreType.DMA((NTM,)),
            ],
            compiler_params=pltpu.CompilerParams(
                vmem_limit_bytes=100 * 1024 * 1024,
                flags=FLAGS,
            ),
        )(A_x, A_k_cache, A_v_cache, A_wq, A_wo, B_w_gate, B_w_up, B_w_down, c, w_mod)
    return fn


_impl = _build(CUT=0,RS=[64,128,192,128]+[256]*5+[128,64,64],BC=1)


@jax.jit
def pallas_adaLN_cond__mha_block_cached__geglu_ffn__prompt_kernel(
    A_x, A_k_cache, A_v_cache, A_wq, A_wo, B_x, B_w_gate, B_w_up, B_w_down, c, w_mod,
):
    return _impl(A_x, A_k_cache, A_v_cache, A_wq, A_wo, B_x, B_w_gate, B_w_up, B_w_down, c, w_mod)
```

```python
import contextlib
import math
import jax
import jax.numpy as jnp
from jax import lax
from jax.experimental import pallas as pl
from jax.experimental.pallas import tpu as pltpu

S, D, H, DH, SK, F = 2048, 512, 32, 128, 2048, 1792
NB = D // 128
EPS = 1e-5
LOG2E = 1.4426950408889634
QSCALE = (DH ** -0.5) * LOG2E
BF, F32, U32 = jnp.bfloat16, jnp.float32, jnp.uint32


def _ln(x):
    m = jnp.mean(x, axis=-1, keepdims=True)
    xc = x - m
    v = jnp.mean(xc * xc, axis=-1, keepdims=True)
    return xc * lax.rsqrt(v + EPS)


def _recip(l):
    r = pl.reciprocal(l, approx=True)
    return r + r * (1.0 - l * r)


def _gelu(x):
    c = math.sqrt(2.0 / math.pi)
    return 0.5 * x * (1.0 + jnp.tanh(c * (x + 0.044715 * (x * x * x))))


def _build(RS=(128, 128, 192, 112, 224, 256, 240, 256, 256, 128, 64, 64), OPLAG=2, ORDER='kqov',
         TM=512, DEP=(('g', 3), ('g', 6), ('g', 9), ('g', 12)), OSP=4, XC=8,
         STAGES=None, ITEMS=None, SCOPES=False, NOFFN=False, FLAGS=None):
    RS = list(RS)
    assert sum(RS) == S
    RMAX, NT = max(RS), len(RS)
    R0 = [sum(RS[:j]) for j in range(NT)]
    XR, NTM = S // XC, S // TM
    scope = (lambda n: jax.named_scope(n)) if SCOPES else (lambda n: contextlib.nullcontext())
    ITEMS = ITEMS or ([('x', j) for j in range(XC)] + [('wq', 0), ('k', 0), ('v', 0), ('wq', 1), ('wo', 0)])
    STAGES = STAGES or ([1, 2] + [1] * XC)

    def kernel(x_hbm, k_hbm, v_hbm, wq_hbm, wo_hbm, wg_hbm, wu_hbm, wd_hbm, c_hbm, wm_hbm,
               o_hbm,
               x_s, kb, vb, wq_s, wo_s, wg_s, wu_s, wd_s, c_s, wm_s, h_s, acc_s, mod_s, o_s,
               q0_s, oc_s, hn_s, zero_s,
               kv_sem, x_sem, w_sem, o_sem):

        def k_copy(head, slot):
            return pltpu.make_async_copy(k_hbm.at[0, head], kb.at[slot], kv_sem.at[slot])

        def v_copy(head, slot):
            return pltpu.make_async_copy(v_hbm.at[0, head], vb.at[slot], kv_sem.at[2 + slot])

        def wq_copy(head, dst):
            col = pl.ds(pl.multiple_of(head * DH, DH), DH)
            return pltpu.make_async_copy(wq_hbm.at[:, col], wq_s.at[dst], w_sem.at[6])

        def wo_copies(head, dst):
            row = pl.ds(pl.multiple_of(head * DH, DH), DH)
            return [pltpu.make_async_copy(wo_hbm.at[row, b * 128:(b + 1) * 128], wo_s.at[dst, b], w_sem.at[7])
                    for b in range(NB)]

        c_cp = pltpu.make_async_copy(c_hbm, c_s, w_sem.at[0])
        wma_cp = pltpu.make_async_copy(wm_hbm.at[:, 0:2 * D], wm_s.at[:, 0:2 * D], w_sem.at[1])
        wmb_cp = pltpu.make_async_copy(wm_hbm.at[:, 2 * D:6 * D], wm_s.at[:, 2 * D:6 * D], w_sem.at[2])
        wg_cp = pltpu.make_async_copy(wg_hbm, wg_s, w_sem.at[3])
        wu_cp = pltpu.make_async_copy(wu_hbm, wu_s, w_sem.at[4])
        wd_cp = pltpu.make_async_copy(wd_hbm, wd_s, w_sem.at[5])
        x_cps = [pltpu.make_async_copy(x_hbm.at[0, i * XR:(i + 1) * XR, :], x_s.at[i * XR:(i + 1) * XR, :],
                                       x_sem.at[i]) for i in range(XC)]

        def item_copies(it):
            kind, j = it
            if kind == 'x':
                return [x_cps[j]]
            if kind == 'wq':
                return [wq_copy(j, j)]
            if kind == 'k':
                return [k_copy(j, j)]
            if kind == 'v':
                return [v_copy(j, j)]
            return wo_copies(j, j + 1)

        pos = [0]

        def issue(n):
            for it in ITEMS[pos[0]:pos[0] + n]:
                for cp in item_copies(it):
                    cp.start()
            pos[0] = min(len(ITEMS), pos[0] + n)

        c_cp.start()
        wma_cp.start()
        issue(STAGES[0])

        wo_s[0] = jnp.zeros((NB, DH, 128), BF)
        oc_s[...] = jnp.zeros(oc_s.shape, BF)
        zero_s[...] = jnp.zeros(zero_s.shape, U32)
        acc_s[...] = jnp.zeros(acc_s.shape, F32)

        with scope('wait_c'):
            c_cp.wait()
        cv = c_s[...].astype(F32)
        sc = jnp.broadcast_to(cv * jax.nn.sigmoid(cv), (16, D)).astype(BF)
        with scope('wait_wma'):
            wma_cp.wait()
        issue(STAGES[1])
        mod_a = jnp.dot(sc, wm_s[:, 0:2 * D], preferred_element_type=F32)
        mod_s[0:1, :] = mod_a[0:1, 0:D]
        mod_s[1:2, :] = 1.0 + mod_a[0:1, D:2 * D]

        with scope('ln'):
            for j in range(XC):
                x_cps[j].wait()
                issue(STAGES[2 + j] if j < XC - 1 else len(ITEMS))
                xv = x_s[j * XR:(j + 1) * XR, :].astype(F32)
                hb = (_ln(xv) * mod_s[1:2, :] + mod_s[0:1, :]).astype(BF)
                for b in range(NB):
                    h_s[b, j * (XR // 2):(j + 1) * (XR // 2), :] = pltpu.bitcast(hb[:, b * 128:(b + 1) * 128], U32)

        def ldw(ref):
            return pltpu.bitcast(ref.bitcast(U32)[...], BF)

        def qp(j, wq_ref):
            r2 = pl.ds(R0[j] // 2, RS[j] // 2)
            hh = jnp.concatenate([pltpu.bitcast(h_s[b, r2, :], BF) for b in range(NB)], axis=1)
            q = jnp.dot(hh, ldw(wq_ref), preferred_element_type=F32)
            return (q * QSCALE).astype(BF)

        def op(j, o, wo_ref):
            w = jnp.concatenate([ldw(wo_ref.at[b]) for b in range(NB)], axis=1)
            acc_s[R0[j]:R0[j] + RS[j], :] += jnp.dot(o, w, preferred_element_type=F32)

        with scope('wait_wq'):
            wq_copy(0, 0).wait()
        q0_s[0:RS[0], :] = qp(0, wq_s.at[0])
        with scope('wait_h0'):
            k_copy(0, 0).wait()
            v_copy(0, 0).wait()
            wq_copy(0, 1).wait()
            for cp in wo_copies(0, 1):
                cp.wait()
        k_copy(1, 1).start()
        wmb_cp.start()
        wg_cp.start()
        wu_cp.start()
        wd_cp.start()

        def head_body(h, carry):
            slot = lax.rem(h, 2)
            hn = jnp.minimum(h + 1, H - 1)
            v_copy(hn, 1 - slot).start()
            wq_copy(jnp.minimum(h + 2, H - 1), h + 2).start()
            for cp in wo_copies(hn, h + 2):
                cp.start()
            k_ref, v_ref = kb.at[slot], vb.at[slot]

            qs = {0: q0_s[0:RS[0], :]}
            os_ = {j - OPLAG: oc_s[j, 0:RS[NT - OPLAG + j], :] for j in range(OPLAG)}
            ss = {}
            for t in range(NT):
                for st in ORDER:
                    if st == 'k':
                        s = lax.dot_general(qs[t], ldw(k_ref), (((1,), (1,)), ((), ())),
                                            preferred_element_type=F32)
                        ss[t] = (s, jnp.max(s, axis=-1, keepdims=True))
                        if t == NT - 1:
                            k_copy(jnp.minimum(h + 2, H - 1), slot).start()
                    elif st == 'q':
                        if t + 1 < NT:
                            qs[t + 1] = qp(t + 1, wq_s.at[h])
                        else:
                            q0_s[0:RS[0], :] = qp(0, wq_s.at[h + 1])
                    elif st == 'o':
                        j = t - OPLAG
                        op(j % NT, os_[j], wo_s.at[h + 1] if j >= 0 else wo_s.at[h])
                    elif st == 'v':
                        s, m = ss[t]
                        p = jnp.exp2(s - m)
                        l = jnp.sum(p, axis=-1, keepdims=True)
                        o = jnp.dot(p.astype(BF), ldw(v_ref), preferred_element_type=F32)
                        os_[t] = (o * _recip(l)).astype(BF)
                        if t >= NT - OPLAG:
                            oc_s[t - (NT - OPLAG), 0:RS[t], :] = os_[t]

            k_copy(0, 1 - slot).wait()
            v_copy(0, 1 - slot).wait()
            wq_copy(0, h + 2).wait()
            for cp in wo_copies(0, h + 2):
                cp.wait()
            return carry

        with scope('heads'):
            lax.fori_loop(0, H, head_body, 0)
        for j in range(OPLAG):
            jj = NT - OPLAG + j
            op(jj, oc_s[j, 0:RS[jj], :], wo_s.at[H])

        wmb_cp.wait()
        wg_cp.wait()
        wu_cp.wait()
        wd_cp.wait()
        if NOFFN:
            o_s[...] = acc_s[...].astype(BF)
            cp = pltpu.make_async_copy(o_s, o_hbm.at[0], o_sem.at[0])
            cp.start()
            k_copy(0, (H - 1) % 2).wait()
            cp.wait()
            return

        mod_b = jnp.dot(sc, wm_s[:, 2 * D:6 * D], preferred_element_type=F32)
        mod_s[2:3, :] = mod_b[0:1, 0:D]
        mod_s[3:4, :] = mod_b[0:1, D:2 * D]
        mod_s[4:5, :] = 1.0 + mod_b[0:1, 2 * D:3 * D]
        mod_s[5:6, :] = mod_b[0:1, 3 * D:4 * D]

        def resid(r):
            return x_s[r, :].astype(F32) + mod_s[2:3, :] * acc_s[r, :]

        def h2_blocks(r0, n):
            r = pl.ds(pl.multiple_of(r0, n), n)
            hb = (_ln(resid(r)) * mod_s[4:5, :] + mod_s[3:4, :]).astype(BF)
            return [pltpu.bitcast(hb[:, b * 128:(b + 1) * 128], U32) for b in range(NB)]

        for b, blk in enumerate(h2_blocks(0, TM)):
            h_s[b, 0:TM // 2, :] = blk

        def ffn_body(i, carry):
            r = pl.ds(pl.multiple_of(i * TM, TM), TM)
            r2 = pl.ds(pl.multiple_of(i * (TM // 2), TM // 2), TM // 2)
            h2 = jnp.concatenate([pltpu.bitcast(h_s[b, r2, :], BF) for b in range(NB)], axis=1)
            inext = lax.rem(i + 1, NTM)
            RC = TM // len(DEP)
            zs = []
            for ch in range(len(DEP)):
                blks = h2_blocks(inext * TM + ch * RC, RC)
                z = None
                for rr in range(RC // 16):
                    for b in range(NB):
                        piece = blks[b][rr * 8:(rr + 1) * 8, :]
                        z = piece if z is None else (z | piece)
                zs.append(z & zero_s[...])
                for b in range(NB):
                    hn_s[b, ch * RC // 2:(ch + 1) * RC // 2, :] = blks[b]

            def dep_weights(w_ref, which):
                parts, c_pos = [], 0
                for ch, (wh, cb) in enumerate(DEP):
                    if wh != which:
                        continue
                    c0 = cb * 128
                    if c0 > c_pos:
                        parts.append(w_ref[:, c_pos:c0])
                    parts.append(pltpu.bitcast(pltpu.bitcast(w_ref[:, c0:c0 + 128], U32)
                                               | jnp.tile(zs[ch], (D // 16, 1)), BF))
                    c_pos = c0 + 128
                if c_pos < F:
                    parts.append(w_ref[:, c_pos:])
                return jnp.concatenate(parts, axis=1) if len(parts) > 1 else parts[0]

            g = jnp.dot(h2, dep_weights(wg_s, 'g'), preferred_element_type=F32)
            u = jnp.dot(h2, dep_weights(wu_s, 'u'), preferred_element_type=F32)
            a = (_gelu(g) * u).astype(BF)
            y = jnp.dot(a, wd_s[...], preferred_element_type=F32)
            res = (resid(r) + mod_s[5:6, :] * y).astype(BF)
            PR = TM // OSP
            for pz in range(OSP):
                rp = pl.ds(pl.multiple_of(i * TM + pz * PR, PR), PR)
                o_s[rp, :] = res[pz * PR:(pz + 1) * PR]
                pltpu.make_async_copy(o_s.at[rp, :], o_hbm.at[0, rp, :], o_sem.at[0]).start()
            r2n = pl.ds(pl.multiple_of(inext * (TM // 2), TM // 2), TM // 2)
            for b in range(NB):
                h_s[b, r2n, :] = hn_s[b]
            return carry

        with scope('ffn'):
            lax.fori_loop(0, NTM, ffn_body, 0)
        with scope('wait_out'):
            k_copy(0, (H - 1) % 2).wait()
            pltpu.make_async_copy(o_s, o_hbm.at[0], o_sem.at[0]).wait()

    @jax.jit
    def fn(A_x, A_k_cache, A_v_cache, A_wq, A_wo, B_x, B_w_gate, B_w_up, B_w_down, c, w_mod):
        any_spec = pl.BlockSpec(memory_space=pl.ANY)
        return pl.pallas_call(
            kernel,
            in_specs=[any_spec] * 10,
            out_specs=any_spec,
            out_shape=jax.ShapeDtypeStruct((1, S, D), A_x.dtype),
            scratch_shapes=[
                pltpu.VMEM((S, D), BF),
                pltpu.VMEM((2, SK, DH), BF),
                pltpu.VMEM((2, SK, DH), BF),
                pltpu.VMEM((H + 2, D, DH), BF),
                pltpu.VMEM((H + 2, NB, DH, 128), BF),
                pltpu.VMEM((D, F), BF),
                pltpu.VMEM((D, F), BF),
                pltpu.VMEM((F, D), BF),
                pltpu.VMEM((1, D), BF),
                pltpu.VMEM((D, 6 * D), BF),
                pltpu.VMEM((NB, S // 2, 128), U32),
                pltpu.VMEM((S, D), F32),
                pltpu.VMEM((8, D), F32),
                pltpu.VMEM((S, D), BF),
                pltpu.VMEM((RMAX, DH), BF),
                pltpu.VMEM((OPLAG, RMAX, DH), BF),
                pltpu.VMEM((NB, TM // 2, 128), U32),
                pltpu.VMEM((8, 128), U32),
                pltpu.SemaphoreType.DMA((4,)),
                pltpu.SemaphoreType.DMA((XC,)),
                pltpu.SemaphoreType.DMA((8,)),
                pltpu.SemaphoreType.DMA((1,)),
            ],
            compiler_params=pltpu.CompilerParams(
                vmem_limit_bytes=100 * 1024 * 1024,
                flags=FLAGS,
            ),
        )(A_x, A_k_cache, A_v_cache, A_wq, A_wo, B_w_gate, B_w_up, B_w_down, c, w_mod)
    return fn


_impl = _build(STAGES=[1,2]+[2]*8)


@jax.jit
def pallas_adaLN_cond__mha_block_cached__geglu_ffn__prompt_kernel(
    A_x, A_k_cache, A_v_cache, A_wq, A_wo, B_x, B_w_gate, B_w_up, B_w_down, c, w_mod,
):
    return _impl(A_x, A_k_cache, A_v_cache, A_wq, A_wo, B_x, B_w_gate, B_w_up, B_w_down, c, w_mod)
```

```python
import contextlib
import math
import jax
import jax.numpy as jnp
from jax import lax
from jax.experimental import pallas as pl
from jax.experimental.pallas import tpu as pltpu

S, D, H, DH, SK, F = 2048, 512, 32, 128, 2048, 1792
NB = D // 128
EPS = 1e-5
LOG2E = 1.4426950408889634
QSCALE = (DH ** -0.5) * LOG2E
BF, F32, U32 = jnp.bfloat16, jnp.float32, jnp.uint32


def _ln(x):
    m = jnp.mean(x, axis=-1, keepdims=True)
    xc = x - m
    v = jnp.mean(xc * xc, axis=-1, keepdims=True)
    return xc * lax.rsqrt(v + EPS)


def _recip(l):
    r = pl.reciprocal(l, approx=True)
    return r + r * (1.0 - l * r)


def _gelu(x):
    c = math.sqrt(2.0 / math.pi)
    return 0.5 * x * (1.0 + jnp.tanh(c * (x + 0.044715 * (x * x * x))))


def _build(RS=(128, 128, 192, 112, 224, 256, 240, 256, 256, 128, 64, 64), OPLAG=2, ORDER='kqov',
         TM=512, DEP=(('g', 3), ('g', 6), ('g', 9), ('g', 12)), OSP=4, XC=8,
         STAGES=None, ITEMS=None, SCOPES=False, NOFFN=False, FLAGS=None, DPOS=None, NOBC=False, NOSC=False, EPI=0, LN0C=1):
    RS = list(RS)
    assert sum(RS) == S
    RMAX, NT = max(RS), len(RS)
    R0 = [sum(RS[:j]) for j in range(NT)]
    XR, NTM = S // XC, S // TM
    scope = (lambda n: jax.named_scope(n)) if SCOPES else (lambda n: contextlib.nullcontext())
    ITEMS = ITEMS or ([('x', j) for j in range(XC)] + [('wq', 0), ('k', 0), ('v', 0), ('wq', 1), ('wo', 0)])
    STAGES = STAGES or ([1, 2] + [1] * XC)

    def kernel(x_hbm, k_hbm, v_hbm, wq_hbm, wo_hbm, wg_hbm, wu_hbm, wd_hbm, c_hbm, wm_hbm,
               o_hbm,
               x_s, kb, vb, wq_s, wo_s, wg_s, wu_s, wd_s, c_s, wm_s, h_s, acc_s, mod_s, o_s,
               q0_s, oc_s, hn_s, zero_s,
               kv_sem, x_sem, w_sem, o_sem):

        def k_copy(head, slot):
            return pltpu.make_async_copy(k_hbm.at[0, head], kb.at[slot], kv_sem.at[slot])

        def v_copy(head, slot):
            return pltpu.make_async_copy(v_hbm.at[0, head], vb.at[slot], kv_sem.at[2 + slot])

        def wq_copy(head, dst):
            col = pl.ds(pl.multiple_of(head * DH, DH), DH)
            return pltpu.make_async_copy(wq_hbm.at[:, col], wq_s.at[dst], w_sem.at[6])

        def wo_copies(head, dst):
            row = pl.ds(pl.multiple_of(head * DH, DH), DH)
            return [pltpu.make_async_copy(wo_hbm.at[row, b * 128:(b + 1) * 128], wo_s.at[dst, b], w_sem.at[7])
                    for b in range(NB)]

        c_cp = pltpu.make_async_copy(c_hbm, c_s, w_sem.at[0])
        wma_cp = pltpu.make_async_copy(wm_hbm.at[:, 0:2 * D], wm_s.at[:, 0:2 * D], w_sem.at[1])
        wmb_cp = pltpu.make_async_copy(wm_hbm.at[:, 2 * D:6 * D], wm_s.at[:, 2 * D:6 * D], w_sem.at[2])
        wg_cp = pltpu.make_async_copy(wg_hbm, wg_s, w_sem.at[3])
        wu_cp = pltpu.make_async_copy(wu_hbm, wu_s, w_sem.at[4])
        wd_cp = pltpu.make_async_copy(wd_hbm, wd_s, w_sem.at[5])
        x_cps = [pltpu.make_async_copy(x_hbm.at[0, i * XR:(i + 1) * XR, :], x_s.at[i * XR:(i + 1) * XR, :],
                                       x_sem.at[i]) for i in range(XC)]

        def item_copies(it):
            kind, j = it
            if kind == 'x':
                return [x_cps[j]]
            if kind == 'wq':
                return [wq_copy(j, j)]
            if kind == 'k':
                return [k_copy(j, j)]
            if kind == 'v':
                return [v_copy(j, j)]
            return wo_copies(j, j + 1)

        pos = [0]

        def issue(n):
            for it in ITEMS[pos[0]:pos[0] + n]:
                for cp in item_copies(it):
                    cp.start()
            pos[0] = min(len(ITEMS), pos[0] + n)

        c_cp.start()
        wma_cp.start()
        issue(STAGES[0])

        wo_s[0] = jnp.zeros((NB, DH, 128), BF)
        oc_s[...] = jnp.zeros(oc_s.shape, BF)
        zero_s[...] = jnp.zeros(zero_s.shape, U32)
        acc_s[...] = jnp.zeros(acc_s.shape, F32)

        with scope('wait_c'):
            c_cp.wait()
        cv = c_s[...].astype(F32)
        sc = jnp.broadcast_to(cv * jax.nn.sigmoid(cv), (16, D)).astype(BF)
        with scope('wait_wma'):
            wma_cp.wait()
        issue(STAGES[1])
        mod_a = jnp.dot(sc, wm_s[:, 0:2 * D], preferred_element_type=F32)
        mod_s[0:1, :] = mod_a[0:1, 0:D]
        mod_s[1:2, :] = 1.0 + mod_a[0:1, D:2 * D]

        with scope('ln'):
            for j in range(XC):
                x_cps[j].wait()
                issue(STAGES[2 + j] if j < XC - 1 else len(ITEMS))
                xv = x_s[j * XR:(j + 1) * XR, :].astype(F32)
                hb = (_ln(xv) * mod_s[1:2, :] + mod_s[0:1, :]).astype(BF)
                for b in range(NB):
                    h_s[b, j * (XR // 2):(j + 1) * (XR // 2), :] = pltpu.bitcast(hb[:, b * 128:(b + 1) * 128], U32)

        def ldw(ref):
            return pltpu.bitcast(ref.bitcast(U32)[...], BF)

        def qp(j, wq_ref):
            r2 = pl.ds(R0[j] // 2, RS[j] // 2)
            hh = jnp.concatenate([pltpu.bitcast(h_s[b, r2, :], BF) for b in range(NB)], axis=1)
            q = jnp.dot(hh, ldw(wq_ref), preferred_element_type=F32)
            return (q * QSCALE).astype(BF)

        def op(j, o, wo_ref):
            w = jnp.concatenate([ldw(wo_ref.at[b]) for b in range(NB)], axis=1)
            acc_s[R0[j]:R0[j] + RS[j], :] += jnp.dot(o, w, preferred_element_type=F32)

        with scope('wait_wq'):
            wq_copy(0, 0).wait()
        q0_s[0:RS[0], :] = qp(0, wq_s.at[0])
        with scope('wait_h0'):
            k_copy(0, 0).wait()
            v_copy(0, 0).wait()
            wq_copy(0, 1).wait()
            for cp in wo_copies(0, 1):
                cp.wait()
        k_copy(1, 1).start()
        wmb_cp.start()
        wg_cp.start()
        wu_cp.start()
        wd_cp.start()

        def head_body(h, carry):
            slot = lax.rem(h, 2)
            hn = jnp.minimum(h + 1, H - 1)


            def prefetch():
                v_copy(hn, 1 - slot).start()
                wq_copy(jnp.minimum(h + 2, H - 1), h + 2).start()
                for cp in wo_copies(hn, h + 2):
                    cp.start()
            if DPOS is None:
                prefetch()
            k_ref, v_ref = kb.at[slot], vb.at[slot]

            qs = {0: q0_s[0:RS[0], :]}
            os_ = {j - OPLAG: oc_s[j, 0:RS[NT - OPLAG + j], :] for j in range(OPLAG)}
            ss = {}
            for t in range(NT):
                for st in ORDER:
                    if st == 'k':
                        s = lax.dot_general(qs[t], ldw(k_ref), (((1,), (1,)), ((), ())),
                                            preferred_element_type=F32)
                        ss[t] = (s, jnp.max(s, axis=-1, keepdims=True))
                        if t == NT - 1:
                            k_copy(jnp.minimum(h + 2, H - 1), slot).start()
                        if DPOS == ('k', t):
                            prefetch()
                    elif st == 'q':
                        if t + 1 < NT:
                            qs[t + 1] = qp(t + 1, wq_s.at[h])
                        else:
                            q0_s[0:RS[0], :] = qp(0, wq_s.at[h + 1])
                        if DPOS == ('q', t):
                            prefetch()
                    elif st == 'o':
                        j = t - OPLAG
                        op(j % NT, os_[j], wo_s.at[h + 1] if j >= 0 else wo_s.at[h])
                        if DPOS == ('o', t):
                            prefetch()
                    elif st == 'v':
                        s, m = ss[t]
                        p = jnp.exp2(s - m)
                        l = jnp.sum(p, axis=-1, keepdims=True)
                        o = jnp.dot(p.astype(BF), ldw(v_ref), preferred_element_type=F32)
                        os_[t] = (o * _recip(l)).astype(BF)
                        if t >= NT - OPLAG:
                            oc_s[t - (NT - OPLAG), 0:RS[t], :] = os_[t]

            k_copy(0, 1 - slot).wait()
            v_copy(0, 1 - slot).wait()
            wq_copy(0, h + 2).wait()
            pltpu.make_async_copy(wo_s.at[h + 2], wo_s.at[h + 2], w_sem.at[7]).wait()
            return carry

        with scope('heads'):
            lax.fori_loop(0, H, head_body, 0)
        for j in range(OPLAG):
            jj = NT - OPLAG + j
            op(jj, oc_s[j, 0:RS[jj], :], wo_s.at[H])

        wmb_cp.wait()
        wg_cp.wait()
        wu_cp.wait()
        wd_cp.wait()
        if NOFFN:
            o_s[...] = acc_s[...].astype(BF)
            cp = pltpu.make_async_copy(o_s, o_hbm.at[0], o_sem.at[0])
            cp.start()
            k_copy(0, (H - 1) % 2).wait()
            cp.wait()
            return

        if EPI == 0:
            mod_b = jnp.dot(sc, wm_s[:, 2 * D:6 * D], preferred_element_type=F32)
            ga, sb = mod_b[0:1, 0:D], mod_b[0:1, D:2 * D]
            cb1, gb = 1.0 + mod_b[0:1, 2 * D:3 * D], mod_b[0:1, 3 * D:4 * D]
        else:
            ga = jnp.dot(sc, wm_s[:, 2 * D:3 * D], preferred_element_type=F32)[0:1, :]
            mod_r = jnp.dot(sc, wm_s[:, 3 * D:6 * D], preferred_element_type=F32)
            sb, cb1, gb = mod_r[0:1, 0:D], 1.0 + mod_r[0:1, D:2 * D], mod_r[0:1, 2 * D:3 * D]

        def resid(r, ga_):
            return x_s[r, :].astype(F32) + ga_ * acc_s[r, :]

        def h2_blocks(r0, n, ga_, sb_, cb1_):
            r = pl.ds(pl.multiple_of(r0, n), n)
            hb = (_ln(resid(r, ga_)) * cb1_ + sb_).astype(BF)
            return [pltpu.bitcast(hb[:, b * 128:(b + 1) * 128], U32) for b in range(NB)]

        C0 = TM // LN0C
        for ch in range(LN0C):
            for b, blk in enumerate(h2_blocks(ch * C0, C0, ga, sb, cb1)):
                h_s[b, ch * C0 // 2:(ch + 1) * C0 // 2, :] = blk
        mod_s[2:3, :] = ga
        mod_s[3:4, :] = sb
        mod_s[4:5, :] = cb1
        mod_s[5:6, :] = gb

        def ffn_body(i, carry):
            r = pl.ds(pl.multiple_of(i * TM, TM), TM)
            r2 = pl.ds(pl.multiple_of(i * (TM // 2), TM // 2), TM // 2)
            h2 = jnp.concatenate([pltpu.bitcast(h_s[b, r2, :], BF) for b in range(NB)], axis=1)
            inext = lax.rem(i + 1, NTM)
            RC = TM // len(DEP)
            zs = []
            for ch in range(len(DEP)):
                blks = h2_blocks(inext * TM + ch * RC, RC, mod_s[2:3, :], mod_s[3:4, :], mod_s[4:5, :])
                z = None
                for rr in range(RC // 16):
                    for b in range(NB):
                        piece = blks[b][rr * 8:(rr + 1) * 8, :]
                        z = piece if z is None else (z | piece)
                zs.append(z & zero_s[...])
                for b in range(NB):
                    hn_s[b, ch * RC // 2:(ch + 1) * RC // 2, :] = blks[b]

            def dep_weights(w_ref, which):
                parts, c_pos = [], 0
                for ch, (wh, cb) in enumerate(DEP):
                    if wh != which:
                        continue
                    c0 = cb * 128
                    if c0 > c_pos:
                        parts.append(w_ref[:, c_pos:c0])
                    parts.append(pltpu.bitcast(pltpu.bitcast(w_ref[:, c0:c0 + 128], U32)
                                               | jnp.tile(zs[ch], (D // 16, 1)), BF))
                    c_pos = c0 + 128
                if c_pos < F:
                    parts.append(w_ref[:, c_pos:])
                return jnp.concatenate(parts, axis=1) if len(parts) > 1 else parts[0]

            g = jnp.dot(h2, dep_weights(wg_s, 'g'), preferred_element_type=F32)
            u = jnp.dot(h2, dep_weights(wu_s, 'u'), preferred_element_type=F32)
            a = (_gelu(g) * u).astype(BF)
            y = jnp.dot(a, wd_s[...], preferred_element_type=F32)
            res = (resid(r, mod_s[2:3, :]) + mod_s[5:6, :] * y).astype(BF)
            PR = TM // OSP
            for pz in range(OSP):
                rp = pl.ds(pl.multiple_of(i * TM + pz * PR, PR), PR)
                o_s[rp, :] = res[pz * PR:(pz + 1) * PR]
                pltpu.make_async_copy(o_s.at[rp, :], o_hbm.at[0, rp, :], o_sem.at[0]).start()
            r2n = pl.ds(pl.multiple_of(inext * (TM // 2), TM // 2), TM // 2)
            for b in range(NB):
                h_s[b, r2n, :] = hn_s[b]
            return carry

        with scope('ffn'):
            lax.fori_loop(0, NTM, ffn_body, 0)
        with scope('wait_out'):
            k_copy(0, (H - 1) % 2).wait()
            pltpu.make_async_copy(o_s, o_hbm.at[0], o_sem.at[0]).wait()

    @jax.jit
    def fn(A_x, A_k_cache, A_v_cache, A_wq, A_wo, B_x, B_w_gate, B_w_up, B_w_down, c, w_mod):
        any_spec = pl.BlockSpec(memory_space=pl.ANY)
        return pl.pallas_call(
            kernel,
            in_specs=[any_spec] * 10,
            out_specs=any_spec,
            out_shape=jax.ShapeDtypeStruct((1, S, D), A_x.dtype),
            scratch_shapes=[
                pltpu.VMEM((S, D), BF),
                pltpu.VMEM((2, SK, DH), BF),
                pltpu.VMEM((2, SK, DH), BF),
                pltpu.VMEM((H + 2, D, DH), BF),
                pltpu.VMEM((H + 2, NB, DH, 128), BF),
                pltpu.VMEM((D, F), BF),
                pltpu.VMEM((D, F), BF),
                pltpu.VMEM((F, D), BF),
                pltpu.VMEM((1, D), BF),
                pltpu.VMEM((D, 6 * D), BF),
                pltpu.VMEM((NB, S // 2, 128), U32),
                pltpu.VMEM((S, D), F32),
                pltpu.VMEM((8, D), F32),
                pltpu.VMEM((S, D), BF),
                pltpu.VMEM((RMAX, DH), BF),
                pltpu.VMEM((OPLAG, RMAX, DH), BF),
                pltpu.VMEM((NB, TM // 2, 128), U32),
                pltpu.VMEM((8, 128), U32),
                pltpu.SemaphoreType.DMA((4,)),
                pltpu.SemaphoreType.DMA((XC,)),
                pltpu.SemaphoreType.DMA((8,)),
                pltpu.SemaphoreType.DMA((1,)),
            ],
            compiler_params=pltpu.CompilerParams(
                vmem_limit_bytes=100 * 1024 * 1024,
                flags=FLAGS,
                disable_bounds_checks=NOBC,
                disable_semaphore_checks=NOSC,
            ),
        )(A_x, A_k_cache, A_v_cache, A_wq, A_wo, B_w_gate, B_w_up, B_w_down, c, w_mod)
    return fn


_impl = _build(RS=[128,128,192,112,224,256,240,256,256,128,64,64],NOBC=True,NOSC=True,DPOS=('o',0),EPI=1,LN0C=2,ITEMS=[('wq',1),('wo',0),('x',0),('x',1),('x',2),('x',3),('x',4),('x',5),('wq',0),('x',6),('k',0),('x',7),('v',0)],STAGES=[3,3,2,2,2,1,0,0,0,0])


@jax.jit
def pallas_adaLN_cond__mha_block_cached__geglu_ffn__prompt_kernel(
    A_x, A_k_cache, A_v_cache, A_wq, A_wo, B_x, B_w_gate, B_w_up, B_w_down, c, w_mod,
):
    return _impl(A_x, A_k_cache, A_v_cache, A_wq, A_wo, B_x, B_w_gate, B_w_up, B_w_down, c, w_mod)
```

```python
import math

import jax
import jax.numpy as jnp
from jax import lax
from jax.experimental import pallas as pl
from jax.experimental.pallas import tpu as pltpu

S, D, H, DH, SK, F = 2048, 512, 32, 128, 2048, 1792
NB = D // 128
EPS = 1e-5
QSCALE = (DH ** -0.5) * 1.4426950408889634
BF, F32, U32 = jnp.bfloat16, jnp.float32, jnp.uint32

RS = (128, 128, 192, 112, 224, 256, 240, 256, 256, 128, 64, 64)
NT = len(RS)
R0 = tuple(sum(RS[:j]) for j in range(NT))
OPLAG = 2
XC = 8
XR = S // XC
TM = 512
NTM = S // TM
OSP = 8
DEP = (('g', 1), ('g', 3), ('g', 5), ('g', 7), ('g', 9), ('g', 11), ('g', 13), ('u', 1))
ITEMS = (('wq', 1), ('wo', 0), ('x', 0), ('x', 1), ('x', 2), ('x', 3), ('x', 4), ('x', 5),
         ('wq0', 0), ('x', 6), ('k', 0), ('x', 7), ('v', 0))
STAGES = (3, 3, 2, 2, 2, 1, 0, 0, 0, 0)

assert sum(RS) == S and sum(STAGES) == len(ITEMS)


def _ln(x):
    m = jnp.mean(x, axis=-1, keepdims=True)
    xc = x - m
    v = jnp.mean(xc * xc, axis=-1, keepdims=True)
    return xc * lax.rsqrt(v + EPS)


def _recip(l):
    r = pl.reciprocal(l, approx=True)
    return r + r * (1.0 - l * r)


def _gelu(x):
    c = math.sqrt(2.0 / math.pi)
    return 0.5 * x * (1.0 + jnp.tanh(c * (x + 0.044715 * (x * x * x))))


def _ldw(ref):
    return pltpu.bitcast(ref.bitcast(U32)[...], BF)


def _to_blocks(hb):
    return [pltpu.bitcast(hb[:, b * 128:(b + 1) * 128], U32) for b in range(NB)]


def _kernel(x_hbm, k_hbm, v_hbm, wq_hbm, wo_hbm, wg_hbm, wu_hbm, wd_hbm, c_hbm, wm_hbm,
            o_hbm,
            x_s, kb, vb, wq_s, wo_s, wg_s, wu_s, wd_s, c_s, wm_s, h_s, acc_s, mod_s, o_s,
            q0_s, oc_s, hn_s, zero_s,
            kv_sem, x_sem, w_sem, o_sem):

    def k_copy(head, slot):
        return pltpu.make_async_copy(k_hbm.at[0, head], kb.at[slot], kv_sem.at[slot])

    def v_copy(head, slot):
        return pltpu.make_async_copy(v_hbm.at[0, head], vb.at[slot], kv_sem.at[2 + slot])

    def wq_copy(head, dst, sem=6):
        col = pl.ds(pl.multiple_of(head * DH, DH), DH)
        return pltpu.make_async_copy(wq_hbm.at[:, col], wq_s.at[dst], w_sem.at[sem])

    def wo_copies(head, dst):
        row = pl.ds(pl.multiple_of(head * DH, DH), DH)
        return [pltpu.make_async_copy(wo_hbm.at[row, b * 128:(b + 1) * 128], wo_s.at[dst, b], w_sem.at[7])
                for b in range(NB)]

    def wo_wait(dst):
        pltpu.make_async_copy(wo_s.at[dst], wo_s.at[dst], w_sem.at[7]).wait()

    c_cp = pltpu.make_async_copy(c_hbm, c_s, w_sem.at[0])
    wma_cp = pltpu.make_async_copy(wm_hbm.at[:, 0:2 * D], wm_s.at[:, 0:2 * D], w_sem.at[1])
    wmb_cp = pltpu.make_async_copy(wm_hbm.at[:, 2 * D:6 * D], wm_s.at[:, 2 * D:6 * D], w_sem.at[2])
    wg_cp = pltpu.make_async_copy(wg_hbm, wg_s, w_sem.at[3])
    wu_cp = pltpu.make_async_copy(wu_hbm, wu_s, w_sem.at[4])
    wd_cp = pltpu.make_async_copy(wd_hbm, wd_s, w_sem.at[5])
    x_cps = [pltpu.make_async_copy(x_hbm.at[0, i * XR:(i + 1) * XR, :], x_s.at[i * XR:(i + 1) * XR, :],
                                   x_sem.at[i]) for i in range(XC)]

    def item_copies(kind, j):
        return {'x': lambda: [x_cps[j]],
                'wq0': lambda: [wq_copy(j, j, sem=8)],
                'wq': lambda: [wq_copy(j, j)],
                'k': lambda: [k_copy(j, j)],
                'v': lambda: [v_copy(j, j)],
                'wo': lambda: wo_copies(j, j + 1)}[kind]()

    def issue(stage):
        first = sum(STAGES[:stage])
        for kind, j in ITEMS[first:first + STAGES[stage]]:
            for cp in item_copies(kind, j):
                cp.start()

    c_cp.start()
    wma_cp.start()
    issue(0)

    wo_s[0] = jnp.zeros((NB, DH, 128), BF)
    oc_s[...] = jnp.zeros(oc_s.shape, BF)
    zero_s[...] = jnp.zeros(zero_s.shape, U32)
    acc_s[...] = jnp.zeros(acc_s.shape, F32)

    c_cp.wait()
    cv = c_s[...].astype(F32)
    sc = jnp.broadcast_to(cv * jax.nn.sigmoid(cv), (16, D)).astype(BF)
    wma_cp.wait()
    issue(1)
    mod_a = jnp.dot(sc, wm_s[:, 0:2 * D], preferred_element_type=F32)
    mod_s[0:1, :] = mod_a[0:1, 0:D]
    mod_s[1:2, :] = 1.0 + mod_a[0:1, D:2 * D]

    for j in range(XC):
        x_cps[j].wait()
        issue(2 + j)
        xv = x_s[j * XR:(j + 1) * XR, :].astype(F32)
        hb = (_ln(xv) * mod_s[1:2, :] + mod_s[0:1, :]).astype(BF)
        for b, blk in enumerate(_to_blocks(hb)):
            h_s[b, j * (XR // 2):(j + 1) * (XR // 2), :] = blk

    def load_h(r2):
        return jnp.concatenate([pltpu.bitcast(h_s[b, r2, :], BF) for b in range(NB)], axis=1)

    def qp(t, wq_ref):
        q = jnp.dot(load_h(pl.ds(R0[t] // 2, RS[t] // 2)), _ldw(wq_ref), preferred_element_type=F32)
        return (q * QSCALE).astype(BF)

    def op(t, o, wo_ref):
        w = jnp.concatenate([_ldw(wo_ref.at[b]) for b in range(NB)], axis=1)
        acc_s[R0[t]:R0[t] + RS[t], :] += jnp.dot(o, w, preferred_element_type=F32)

    wq_copy(0, 0, sem=8).wait()
    q0_s[0:RS[0], :] = qp(0, wq_s.at[0])
    k_copy(0, 0).wait()
    v_copy(0, 0).wait()
    wq_copy(0, 1).wait()
    wo_wait(1)
    k_copy(1, 1).start()
    wmb_cp.start()
    wg_cp.start()
    wu_cp.start()
    wd_cp.start()

    def head_body(h, carry):
        slot = lax.rem(h, 2)
        hn = jnp.minimum(h + 1, H - 1)
        hn2 = jnp.minimum(h + 2, H - 1)
        k_ref, v_ref = kb.at[slot], vb.at[slot]

        qs = {0: q0_s[0:RS[0], :]}
        os_ = {j - OPLAG: oc_s[j, 0:RS[NT - OPLAG + j], :] for j in range(OPLAG)}
        for t in range(NT):
            s = lax.dot_general(qs.pop(t), _ldw(k_ref), (((1,), (1,)), ((), ())), preferred_element_type=F32)
            m = jnp.max(s, axis=-1, keepdims=True)
            if t == NT - 1:
                k_copy(hn2, slot).start()
            if t + 1 < NT:
                qs[t + 1] = qp(t + 1, wq_s.at[h])
            else:
                q0_s[0:RS[0], :] = qp(0, wq_s.at[h + 1])
            j = t - OPLAG
            op(j % NT, os_.pop(j), wo_s.at[h + 1] if j >= 0 else wo_s.at[h])
            if t == 0:
                v_copy(hn, 1 - slot).start()
                wq_copy(hn2, h + 2).start()
                for cp in wo_copies(hn, h + 2):
                    cp.start()
            p = jnp.exp2(s - m)
            l = jnp.sum(p, axis=-1, keepdims=True)
            o = jnp.dot(p.astype(BF), _ldw(v_ref), preferred_element_type=F32)
            os_[t] = (o * _recip(l)).astype(BF)
            if t >= NT - OPLAG:
                oc_s[t - (NT - OPLAG), 0:RS[t], :] = os_[t]

        k_copy(0, 1 - slot).wait()
        v_copy(0, 1 - slot).wait()
        wq_copy(0, h + 2).wait()
        wo_wait(h + 2)
        return carry

    lax.fori_loop(0, H, head_body, 0)
    for j in range(OPLAG):
        t = NT - OPLAG + j
        op(t, oc_s[j, 0:RS[t], :], wo_s.at[H])

    wmb_cp.wait()
    wg_cp.wait()
    wu_cp.wait()
    wd_cp.wait()
    ga = jnp.dot(sc, wm_s[:, 2 * D:3 * D], preferred_element_type=F32)[0:1, :]
    mod_r = jnp.dot(sc, wm_s[:, 3 * D:6 * D], preferred_element_type=F32)
    sb, cb1, gb = mod_r[0:1, 0:D], 1.0 + mod_r[0:1, D:2 * D], mod_r[0:1, 2 * D:3 * D]

    def resid(r, ga_):
        return x_s[r, :].astype(F32) + ga_ * acc_s[r, :]

    def h2_blocks(r0, n, ga_, sb_, cb1_):
        r = pl.ds(pl.multiple_of(r0, n), n)
        return _to_blocks((_ln(resid(r, ga_)) * cb1_ + sb_).astype(BF))

    for ch in range(2):
        for b, blk in enumerate(h2_blocks(ch * (TM // 2), TM // 2, ga, sb, cb1)):
            h_s[b, ch * (TM // 4):(ch + 1) * (TM // 4), :] = blk
    mod_s[2:3, :] = ga
    mod_s[3:4, :] = sb
    mod_s[4:5, :] = cb1
    mod_s[5:6, :] = gb

    def ffn_body(i, carry):
        r = pl.ds(pl.multiple_of(i * TM, TM), TM)
        h2 = load_h(pl.ds(pl.multiple_of(i * (TM // 2), TM // 2), TM // 2))
        inext = lax.rem(i + 1, NTM)

        rc = TM // len(DEP)
        zs = []
        for ch in range(len(DEP)):
            blks = h2_blocks(inext * TM + ch * rc, rc, mod_s[2:3, :], mod_s[3:4, :], mod_s[4:5, :])
            z = None
            for rr in range(rc // 16):
                for b in range(NB):
                    piece = blks[b][rr * 8:(rr + 1) * 8, :]
                    z = piece if z is None else (z | piece)
            zs.append(z & zero_s[...])
            for b in range(NB):
                hn_s[b, ch * rc // 2:(ch + 1) * rc // 2, :] = blks[b]

        def tied(w_ref, which):
            parts, pos = [], 0
            for ch, (wh, cb) in enumerate(DEP):
                if wh != which:
                    continue
                c0 = cb * 128
                if c0 > pos:
                    parts.append(w_ref[:, pos:c0])
                blk = pltpu.bitcast(w_ref[:, c0:c0 + 128], U32) | jnp.tile(zs[ch], (D // 16, 1))
                parts.append(pltpu.bitcast(blk, BF))
                pos = c0 + 128
            if pos < F:
                parts.append(w_ref[:, pos:])
            return jnp.concatenate(parts, axis=1)

        g = jnp.dot(h2, tied(wg_s, 'g'), preferred_element_type=F32)
        u = jnp.dot(h2, tied(wu_s, 'u'), preferred_element_type=F32)
        a = (_gelu(g) * u).astype(BF)
        y = jnp.dot(a, wd_s[...], preferred_element_type=F32)
        res = (resid(r, mod_s[2:3, :]) + mod_s[5:6, :] * y).astype(BF)
        pr = TM // OSP
        for pz in range(OSP):
            rp = pl.ds(pl.multiple_of(i * TM + pz * pr, pr), pr)
            o_s[rp, :] = res[pz * pr:(pz + 1) * pr]
            pltpu.make_async_copy(o_s.at[rp, :], o_hbm.at[0, rp, :], o_sem.at[0]).start()
        r2n = pl.ds(pl.multiple_of(inext * (TM // 2), TM // 2), TM // 2)
        for b in range(NB):
            h_s[b, r2n, :] = hn_s[b]
        return carry

    lax.fori_loop(0, NTM, ffn_body, 0)
    k_copy(0, (H - 1) % 2).wait()
    pltpu.make_async_copy(o_s, o_hbm.at[0], o_sem.at[0]).wait()


@jax.jit
def pallas_adaLN_cond__mha_block_cached__geglu_ffn__prompt_kernel(
    A_x: jax.Array,
    A_k_cache: jax.Array,
    A_v_cache: jax.Array,
    A_wq: jax.Array,
    A_wo: jax.Array,
    B_x: jax.Array,
    B_w_gate: jax.Array,
    B_w_up: jax.Array,
    B_w_down: jax.Array,
    c: jax.Array,
    w_mod: jax.Array,
):
    del B_x
    any_spec = pl.BlockSpec(memory_space=pl.ANY)
    return pl.pallas_call(
        _kernel,
        in_specs=[any_spec] * 10,
        out_specs=any_spec,
        out_shape=jax.ShapeDtypeStruct((1, S, D), A_x.dtype),
        scratch_shapes=[
            pltpu.VMEM((S, D), BF),
            pltpu.VMEM((2, SK, DH), BF),
            pltpu.VMEM((2, SK, DH), BF),
            pltpu.VMEM((H + 2, D, DH), BF),
            pltpu.VMEM((H + 2, NB, DH, 128), BF),
            pltpu.VMEM((D, F), BF),
            pltpu.VMEM((D, F), BF),
            pltpu.VMEM((F, D), BF),
            pltpu.VMEM((1, D), BF),
            pltpu.VMEM((D, 6 * D), BF),
            pltpu.VMEM((NB, S // 2, 128), U32),
            pltpu.VMEM((S, D), F32),
            pltpu.VMEM((8, D), F32),
            pltpu.VMEM((S, D), BF),
            pltpu.VMEM((max(RS), DH), BF),
            pltpu.VMEM((OPLAG, max(RS), DH), BF),
            pltpu.VMEM((NB, TM // 2, 128), U32),
            pltpu.VMEM((8, 128), U32),
            pltpu.SemaphoreType.DMA((4,)),
            pltpu.SemaphoreType.DMA((XC,)),
            pltpu.SemaphoreType.DMA((9,)),
            pltpu.SemaphoreType.DMA((1,)),
        ],
        compiler_params=pltpu.CompilerParams(
            vmem_limit_bytes=100 * 1024 * 1024,
            disable_bounds_checks=True,
            disable_semaphore_checks=True,
        ),
    )(A_x, A_k_cache, A_v_cache, A_wq, A_wo, B_w_gate, B_w_up, B_w_down, c, w_mod)
```

```python
import math

import jax
import jax.numpy as jnp
from jax import lax
from jax.experimental import pallas as pl
from jax.experimental.pallas import tpu as pltpu

S, D, H, DH, SK, F = 2048, 512, 32, 128, 2048, 1792
NB = D // 128
EPS = 1e-5
QSCALE = (DH ** -0.5) * 1.4426950408889634
BF, F32, U32 = jnp.bfloat16, jnp.float32, jnp.uint32

RS = (128, 128, 192, 112, 224, 256, 240, 256, 256, 128, 64, 64)
NT = len(RS)
R0 = tuple(sum(RS[:j]) for j in range(NT))
OPLAG = 2
TM = 512
NTM = S // TM
OSP = 8
DEP = (('g', 1), ('g', 3), ('g', 5), ('g', 7), ('g', 9), ('g', 11), ('g', 13), ('u', 1))
TA, TB = 2, 5

assert sum(RS) == S


def _ln(x):
    m = jnp.mean(x, axis=-1, keepdims=True)
    xc = x - m
    v = jnp.mean(xc * xc, axis=-1, keepdims=True)
    return xc * lax.rsqrt(v + EPS)


def _recip(l):
    r = pl.reciprocal(l, approx=True)
    return r + r * (1.0 - l * r)


def _gelu(x):
    c = math.sqrt(2.0 / math.pi)
    return 0.5 * x * (1.0 + jnp.tanh(c * (x + 0.044715 * (x * x * x))))


def _ldw(ref):
    return pltpu.bitcast(ref.bitcast(U32)[...], BF)


def _to_blocks(hb):
    return [pltpu.bitcast(hb[:, b * 128:(b + 1) * 128], U32) for b in range(NB)]


def _kernel(x_hbm, k_hbm, v_hbm, wq_hbm, wo_hbm, wg_hbm, wu_hbm, wd_hbm, c_hbm, wm_hbm,
            o_hbm,
            x_s, kb, vb, wq_s, wo_s, wg_s, wu_s, wd_s, c_s, wm_s, h_s, acc_s, mod_s, o_s,
            q0_s, oc_s, hn_s, zero_s,
            kv_sem, x_sem, w_sem, o_sem):

    def k_copy(head, slot):
        return pltpu.make_async_copy(k_hbm.at[0, head], kb.at[slot], kv_sem.at[slot])

    def v_copy(head, slot):
        return pltpu.make_async_copy(v_hbm.at[0, head], vb.at[slot], kv_sem.at[2 + slot])

    def wq_copy(head, dst, sem=6):
        col = pl.ds(pl.multiple_of(head * DH, DH), DH)
        return pltpu.make_async_copy(wq_hbm.at[:, col], wq_s.at[dst], w_sem.at[sem])

    def wo_copies(head, dst):
        row = pl.ds(pl.multiple_of(head * DH, DH), DH)
        return [pltpu.make_async_copy(wo_hbm.at[row, b * 128:(b + 1) * 128], wo_s.at[dst, b], w_sem.at[7])
                for b in range(NB)]

    def wo_wait(dst):
        pltpu.make_async_copy(wo_s.at[dst], wo_s.at[dst], w_sem.at[7]).wait()

    c_cp = pltpu.make_async_copy(c_hbm, c_s, w_sem.at[0])
    wma_cp = pltpu.make_async_copy(wm_hbm.at[:, 0:2 * D], wm_s.at[:, 0:2 * D], w_sem.at[1])
    wmb_cp = pltpu.make_async_copy(wm_hbm.at[:, 2 * D:6 * D], wm_s.at[:, 2 * D:6 * D], w_sem.at[2])
    wg_cp = pltpu.make_async_copy(wg_hbm, wg_s, w_sem.at[3])
    wu_cp = pltpu.make_async_copy(wu_hbm, wu_s, w_sem.at[4])
    wd_cp = pltpu.make_async_copy(wd_hbm, wd_s, w_sem.at[5])

    def x_copy(lo, hi, sem):
        return pltpu.make_async_copy(x_hbm.at[0, lo:hi, :], x_s.at[lo:hi, :], x_sem.at[sem])

    xa_cp, xb_cp, xc_cp = x_copy(0, R0[TA], 0), x_copy(R0[TA], R0[TB], 1), x_copy(R0[TB], S, 2)

    c_cp.start()
    wma_cp.start()
    xa_cp.start()
    wq_copy(0, 0, sem=8).start()

    zero_s[...] = jnp.zeros(zero_s.shape, U32)
    acc_s[...] = jnp.zeros(acc_s.shape, F32)

    c_cp.wait()
    k_copy(0, 0).start()
    v_copy(0, 0).start()
    cv = c_s[...].astype(F32)
    sc = jnp.broadcast_to(cv * jax.nn.sigmoid(cv), (16, D)).astype(BF)
    wma_cp.wait()
    mod_a = jnp.dot(sc, wm_s[:, 0:2 * D], preferred_element_type=F32)
    mod_s[0:1, :] = mod_a[0:1, 0:D]
    mod_s[1:2, :] = 1.0 + mod_a[0:1, D:2 * D]

    def ln_tile(t):
        xv = x_s[R0[t]:R0[t] + RS[t], :].astype(F32)
        hb = (_ln(xv) * mod_s[1:2, :] + mod_s[0:1, :]).astype(BF)
        for b, blk in enumerate(_to_blocks(hb)):
            h_s[b, R0[t] // 2:(R0[t] + RS[t]) // 2, :] = blk

    xa_cp.wait()
    xb_cp.start()
    for cp in wo_copies(0, 1):
        cp.start()
    for t in range(TA):
        ln_tile(t)

    def load_h(r2):
        return jnp.concatenate([pltpu.bitcast(h_s[b, r2, :], BF) for b in range(NB)], axis=1)

    def qp(t, wq_ref):
        q = jnp.dot(load_h(pl.ds(R0[t] // 2, RS[t] // 2)), _ldw(wq_ref), preferred_element_type=F32)
        return (q * QSCALE).astype(BF)

    def op(t, o, wo_ref):
        w = jnp.concatenate([_ldw(wo_ref.at[b]) for b in range(NB)], axis=1)
        acc_s[R0[t]:R0[t] + RS[t], :] += jnp.dot(o, w, preferred_element_type=F32)

    wq_copy(0, 0, sem=8).wait()
    q0_s[0:RS[0], :] = qp(0, wq_s.at[0])
    k_copy(0, 0).wait()
    v_copy(0, 0).wait()

    def head_body(h, carry, first=False):
        if first:
            slot, hn, hn2 = 0, 1, 2
        else:
            slot = lax.rem(h, 2)
            hn = jnp.minimum(h + 1, H - 1)
            hn2 = jnp.minimum(h + 2, H - 1)
        k_ref, v_ref = kb.at[slot], vb.at[slot]

        def prefetch():
            v_copy(hn, 1 - slot).start()
            wq_copy(hn2, h + 2).start()
            for cp in wo_copies(hn, h + 2):
                cp.start()

        qs = {0: q0_s[0:RS[0], :]}
        os_ = {} if first else {j - OPLAG: oc_s[j, 0:RS[NT - OPLAG + j], :] for j in range(OPLAG)}
        for t in range(NT):
            if first and t + 1 == TA:
                xb_cp.wait()
                wo_wait(1)
                xc_cp.start()
                wq_copy(1, 1).start()
            if first and t + 1 == TB:
                xc_cp.wait()
                wq_copy(1, 1).wait()
                k_copy(1, 1).start()
                prefetch()
                wmb_cp.start()
                wg_cp.start()
                wu_cp.start()
                wd_cp.start()
            s = lax.dot_general(qs.pop(t), _ldw(k_ref), (((1,), (1,)), ((), ())), preferred_element_type=F32)
            m = jnp.max(s, axis=-1, keepdims=True)
            if t == NT - 1:
                k_copy(hn2, slot).start()
            if first and TA <= t + 1 < NT:
                ln_tile(t + 1)
            if t + 1 < NT:
                qs[t + 1] = qp(t + 1, wq_s.at[h])
            else:
                q0_s[0:RS[0], :] = qp(0, wq_s.at[h + 1])
            j = t - OPLAG
            if j >= 0 or not first:
                op(j % NT, os_.pop(j), wo_s.at[h + 1] if j >= 0 else wo_s.at[h])
            if t == 0 and not first:
                prefetch()
            p = jnp.exp2(s - m)
            l = jnp.sum(p, axis=-1, keepdims=True)
            o = jnp.dot(p.astype(BF), _ldw(v_ref), preferred_element_type=F32)
            os_[t] = (o * _recip(l)).astype(BF)
            if t >= NT - OPLAG:
                oc_s[t - (NT - OPLAG), 0:RS[t], :] = os_[t]

        k_copy(0, 1 - slot).wait()
        v_copy(0, 1 - slot).wait()
        wq_copy(0, h + 2).wait()
        wo_wait(h + 2)
        return carry

    head_body(0, 0, first=True)
    lax.fori_loop(1, H, head_body, 0)
    for j in range(OPLAG):
        t = NT - OPLAG + j
        op(t, oc_s[j, 0:RS[t], :], wo_s.at[H])

    wmb_cp.wait()
    wg_cp.wait()
    wu_cp.wait()
    wd_cp.wait()
    ga = jnp.dot(sc, wm_s[:, 2 * D:3 * D], preferred_element_type=F32)[0:1, :]
    mod_r = jnp.dot(sc, wm_s[:, 3 * D:6 * D], preferred_element_type=F32)
    sb, cb1, gb = mod_r[0:1, 0:D], 1.0 + mod_r[0:1, D:2 * D], mod_r[0:1, 2 * D:3 * D]

    def resid(r, ga_):
        return x_s[r, :].astype(F32) + ga_ * acc_s[r, :]

    def h2_blocks(r0, n, ga_, sb_, cb1_):
        r = pl.ds(pl.multiple_of(r0, n), n)
        return _to_blocks((_ln(resid(r, ga_)) * cb1_ + sb_).astype(BF))

    for ch in range(2):
        for b, blk in enumerate(h2_blocks(ch * (TM // 2), TM // 2, ga, sb, cb1)):
            h_s[b, ch * (TM // 4):(ch + 1) * (TM // 4), :] = blk
    mod_s[2:3, :] = ga
    mod_s[3:4, :] = sb
    mod_s[4:5, :] = cb1
    mod_s[5:6, :] = gb

    def ffn_body(i, carry):
        r = pl.ds(pl.multiple_of(i * TM, TM), TM)
        h2 = load_h(pl.ds(pl.multiple_of(i * (TM // 2), TM // 2), TM // 2))
        inext = lax.rem(i + 1, NTM)

        rc = TM // len(DEP)
        zs = []
        for ch in range(len(DEP)):
            blks = h2_blocks(inext * TM + ch * rc, rc, mod_s[2:3, :], mod_s[3:4, :], mod_s[4:5, :])
            z = None
            for rr in range(rc // 16):
                for b in range(NB):
                    piece = blks[b][rr * 8:(rr + 1) * 8, :]
                    z = piece if z is None else (z | piece)
            zs.append(z & zero_s[...])
            for b in range(NB):
                hn_s[b, ch * rc // 2:(ch + 1) * rc // 2, :] = blks[b]

        def tied(w_ref, which):
            parts, pos = [], 0
            for ch, (wh, cb) in enumerate(DEP):
                if wh != which:
                    continue
                c0 = cb * 128
                if c0 > pos:
                    parts.append(w_ref[:, pos:c0])
                blk = pltpu.bitcast(w_ref[:, c0:c0 + 128], U32) | jnp.tile(zs[ch], (D // 16, 1))
                parts.append(pltpu.bitcast(blk, BF))
                pos = c0 + 128
            if pos < F:
                parts.append(w_ref[:, pos:])
            return jnp.concatenate(parts, axis=1)

        g = jnp.dot(h2, tied(wg_s, 'g'), preferred_element_type=F32)
        u = jnp.dot(h2, tied(wu_s, 'u'), preferred_element_type=F32)
        a = (_gelu(g) * u).astype(BF)
        y = jnp.dot(a, wd_s[...], preferred_element_type=F32)
        res = (resid(r, mod_s[2:3, :]) + mod_s[5:6, :] * y).astype(BF)
        pr = TM // OSP
        for pz in range(OSP):
            rp = pl.ds(pl.multiple_of(i * TM + pz * pr, pr), pr)
            o_s[rp, :] = res[pz * pr:(pz + 1) * pr]
            pltpu.make_async_copy(o_s.at[rp, :], o_hbm.at[0, rp, :], o_sem.at[0]).start()
        r2n = pl.ds(pl.multiple_of(inext * (TM // 2), TM // 2), TM // 2)
        for b in range(NB):
            h_s[b, r2n, :] = hn_s[b]
        return carry

    lax.fori_loop(0, NTM, ffn_body, 0)
    k_copy(0, (H - 1) % 2).wait()
    pltpu.make_async_copy(o_s, o_hbm.at[0], o_sem.at[0]).wait()


@jax.jit
def pallas_adaLN_cond__mha_block_cached__geglu_ffn__prompt_kernel(
    A_x: jax.Array,
    A_k_cache: jax.Array,
    A_v_cache: jax.Array,
    A_wq: jax.Array,
    A_wo: jax.Array,
    B_x: jax.Array,
    B_w_gate: jax.Array,
    B_w_up: jax.Array,
    B_w_down: jax.Array,
    c: jax.Array,
    w_mod: jax.Array,
):
    del B_x
    any_spec = pl.BlockSpec(memory_space=pl.ANY)
    return pl.pallas_call(
        _kernel,
        in_specs=[any_spec] * 10,
        out_specs=any_spec,
        out_shape=jax.ShapeDtypeStruct((1, S, D), A_x.dtype),
        scratch_shapes=[
            pltpu.VMEM((S, D), BF),
            pltpu.VMEM((2, SK, DH), BF),
            pltpu.VMEM((2, SK, DH), BF),
            pltpu.VMEM((H + 2, D, DH), BF),
            pltpu.VMEM((H + 2, NB, DH, 128), BF),
            pltpu.VMEM((D, F), BF),
            pltpu.VMEM((D, F), BF),
            pltpu.VMEM((F, D), BF),
            pltpu.VMEM((1, D), BF),
            pltpu.VMEM((D, 6 * D), BF),
            pltpu.VMEM((NB, S // 2, 128), U32),
            pltpu.VMEM((S, D), F32),
            pltpu.VMEM((8, D), F32),
            pltpu.VMEM((S, D), BF),
            pltpu.VMEM((max(RS), DH), BF),
            pltpu.VMEM((OPLAG, max(RS), DH), BF),
            pltpu.VMEM((NB, TM // 2, 128), U32),
            pltpu.VMEM((8, 128), U32),
            pltpu.SemaphoreType.DMA((4,)),
            pltpu.SemaphoreType.DMA((3,)),
            pltpu.SemaphoreType.DMA((9,)),
            pltpu.SemaphoreType.DMA((1,)),
        ],
        compiler_params=pltpu.CompilerParams(
            vmem_limit_bytes=100 * 1024 * 1024,
            disable_bounds_checks=True,
            disable_semaphore_checks=True,
        ),
    )(A_x, A_k_cache, A_v_cache, A_wq, A_wo, B_w_gate, B_w_up, B_w_down, c, w_mod)
```

```python
import math

import jax
import jax.numpy as jnp
from jax import lax
from jax.experimental import pallas as pl
from jax.experimental.pallas import tpu as pltpu

S, D, H, DH, SK, F = 2048, 512, 32, 128, 2048, 1792
NB = D // 128
EPS = 1e-5
QSCALE = (DH ** -0.5) * 1.4426950408889634
BF, F32, U32 = jnp.bfloat16, jnp.float32, jnp.uint32

RS = (128, 144, 192, 112, 208, 224, 256, 256, 256, 144, 64, 64)
NT = len(RS)
R0 = tuple(sum(RS[:j]) for j in range(NT))
OPLAG = 2
TM = 512
NTM = S // TM
OSP = 8
DEP = (('g', 1), ('g', 3), ('g', 5), ('g', 7), ('g', 9), ('g', 11), ('g', 13), ('u', 1))
TA, TB = 2, 5

assert sum(RS) == S


def _ln(x):
    m = jnp.mean(x, axis=-1, keepdims=True)
    xc = x - m
    v = jnp.mean(xc * xc, axis=-1, keepdims=True)
    return xc * lax.rsqrt(v + EPS)


def _recip(l):
    r = pl.reciprocal(l, approx=True)
    return r + r * (1.0 - l * r)


def _gelu(x):
    c = math.sqrt(2.0 / math.pi)
    return 0.5 * x * (1.0 + jnp.tanh(c * (x + 0.044715 * (x * x * x))))


def _ldw(ref):
    return pltpu.bitcast(ref.bitcast(U32)[...], BF)


def _to_blocks(hb):
    return [pltpu.bitcast(hb[:, b * 128:(b + 1) * 128], U32) for b in range(NB)]


def _kernel(x_hbm, k_hbm, v_hbm, wq_hbm, wo_hbm, wg_hbm, wu_hbm, wd_hbm, c_hbm, wm_hbm,
            o_hbm,
            x_s, kb, vb, wq_s, wo_s, wg_s, wu_s, wd_s, c_s, wm_s, h_s, acc_s, mod_s, o_s,
            q0_s, oc_s, hn_s, zero_s,
            kv_sem, x_sem, w_sem, o_sem):

    def k_copy(head, slot):
        return pltpu.make_async_copy(k_hbm.at[0, head], kb.at[slot], kv_sem.at[slot])

    def v_copy(head, slot):
        return pltpu.make_async_copy(v_hbm.at[0, head], vb.at[slot], kv_sem.at[2 + slot])

    def wq_copy(head, dst, sem=6):
        col = pl.ds(pl.multiple_of(head * DH, DH), DH)
        return pltpu.make_async_copy(wq_hbm.at[:, col], wq_s.at[dst], w_sem.at[sem])

    def wo_copies(head, dst):
        row = pl.ds(pl.multiple_of(head * DH, DH), DH)
        return [pltpu.make_async_copy(wo_hbm.at[row, b * 128:(b + 1) * 128], wo_s.at[dst, b], w_sem.at[7])
                for b in range(NB)]

    def wo_wait(dst):
        pltpu.make_async_copy(wo_s.at[dst], wo_s.at[dst], w_sem.at[7]).wait()

    c_cp = pltpu.make_async_copy(c_hbm, c_s, w_sem.at[0])
    wma_cp = pltpu.make_async_copy(wm_hbm.at[:, 0:2 * D], wm_s.at[:, 0:2 * D], w_sem.at[1])
    wmb_cp = pltpu.make_async_copy(wm_hbm.at[:, 2 * D:6 * D], wm_s.at[:, 2 * D:6 * D], w_sem.at[2])
    wg_cp = pltpu.make_async_copy(wg_hbm, wg_s, w_sem.at[3])
    wu_cp = pltpu.make_async_copy(wu_hbm, wu_s, w_sem.at[4])
    wd_cp = pltpu.make_async_copy(wd_hbm, wd_s, w_sem.at[5])

    def x_copy(lo, hi, sem):
        return pltpu.make_async_copy(x_hbm.at[0, lo:hi, :], x_s.at[lo:hi, :], x_sem.at[sem])

    xa_cp, xb_cp, xc_cp = x_copy(0, R0[TA], 0), x_copy(R0[TA], R0[TB], 1), x_copy(R0[TB], S, 2)

    c_cp.start()
    wma_cp.start()
    xa_cp.start()
    wq_copy(0, 0, sem=8).start()

    zero_s[...] = jnp.zeros(zero_s.shape, U32)
    acc_s[...] = jnp.zeros(acc_s.shape, F32)

    c_cp.wait()
    k_copy(0, 0).start()
    v_copy(0, 0).start()
    cv = c_s[...].astype(F32)
    sc = jnp.broadcast_to(cv * jax.nn.sigmoid(cv), (16, D)).astype(BF)
    wma_cp.wait()
    mod_a = jnp.dot(sc, wm_s[:, 0:2 * D], preferred_element_type=F32)
    mod_s[0:1, :] = mod_a[0:1, 0:D]
    mod_s[1:2, :] = 1.0 + mod_a[0:1, D:2 * D]

    def ln_tile(t):
        xv = x_s[R0[t]:R0[t] + RS[t], :].astype(F32)
        hb = (_ln(xv) * mod_s[1:2, :] + mod_s[0:1, :]).astype(BF)
        for b, blk in enumerate(_to_blocks(hb)):
            h_s[b, R0[t] // 2:(R0[t] + RS[t]) // 2, :] = blk

    xa_cp.wait()
    xb_cp.start()
    for cp in wo_copies(0, 1):
        cp.start()
    for t in range(TA):
        ln_tile(t)

    def load_h(r2):
        return jnp.concatenate([pltpu.bitcast(h_s[b, r2, :], BF) for b in range(NB)], axis=1)

    def qp(t, wq_ref):
        q = jnp.dot(load_h(pl.ds(R0[t] // 2, RS[t] // 2)), _ldw(wq_ref), preferred_element_type=F32)
        return (q * QSCALE).astype(BF)

    def op(t, o, wo_ref):
        w = jnp.concatenate([_ldw(wo_ref.at[b]) for b in range(NB)], axis=1)
        acc_s[R0[t]:R0[t] + RS[t], :] += jnp.dot(o, w, preferred_element_type=F32)

    wq_copy(0, 0, sem=8).wait()
    q0_s[0:RS[0], :] = qp(0, wq_s.at[0])
    k_copy(0, 0).wait()
    v_copy(0, 0).wait()

    def head_body(h, carry, first=False):
        if first:
            slot, hn, hn2 = 0, 1, 2
        else:
            slot = lax.rem(h, 2)
            hn = jnp.minimum(h + 1, H - 1)
            hn2 = jnp.minimum(h + 2, H - 1)
        k_ref, v_ref = kb.at[slot], vb.at[slot]

        def prefetch():
            v_copy(hn, 1 - slot).start()
            wq_copy(hn2, h + 2).start()
            for cp in wo_copies(hn, h + 2):
                cp.start()

        qs = {0: q0_s[0:RS[0], :]}
        os_ = {} if first else {j - OPLAG: oc_s[j, 0:RS[NT - OPLAG + j], :] for j in range(OPLAG)}
        for t in range(NT):
            if first and t + 1 == TA:
                xb_cp.wait()
                wo_wait(1)
                xc_cp.start()
                wq_copy(1, 1).start()
            if first and t + 1 == TB:
                xc_cp.wait()
                wq_copy(1, 1).wait()
                k_copy(1, 1).start()
                prefetch()
                wmb_cp.start()
                wg_cp.start()
                wu_cp.start()
                wd_cp.start()
            if t < OPLAG and not first:
                op((t - OPLAG) % NT, os_.pop(t - OPLAG), wo_s.at[h])
            s = lax.dot_general(qs.pop(t), _ldw(k_ref), (((1,), (1,)), ((), ())), preferred_element_type=F32)
            m = jnp.max(s, axis=-1, keepdims=True)
            if t == NT - 1:
                k_copy(hn2, slot).start()
            if first and TA <= t + 1 < NT:
                ln_tile(t + 1)
            if t + 1 < NT:
                qs[t + 1] = qp(t + 1, wq_s.at[h])
            else:
                q0_s[0:RS[0], :] = qp(0, wq_s.at[h + 1])
            if t >= OPLAG:
                op(t - OPLAG, os_.pop(t - OPLAG), wo_s.at[h + 1])
            if t == 0 and not first:
                prefetch()
            p = jnp.exp2(s - m)
            l = jnp.sum(p, axis=-1, keepdims=True)
            o = jnp.dot(p.astype(BF), _ldw(v_ref), preferred_element_type=F32)
            os_[t] = (o * _recip(l)).astype(BF)
            if t >= NT - OPLAG:
                oc_s[t - (NT - OPLAG), 0:RS[t], :] = os_[t]

        k_copy(0, 1 - slot).wait()
        v_copy(0, 1 - slot).wait()
        wq_copy(0, h + 2).wait()
        wo_wait(h + 2)
        return carry

    head_body(0, 0, first=True)
    lax.fori_loop(1, H, head_body, 0)
    for j in range(OPLAG):
        t = NT - OPLAG + j
        op(t, oc_s[j, 0:RS[t], :], wo_s.at[H])

    wmb_cp.wait()
    wg_cp.wait()
    wu_cp.wait()
    wd_cp.wait()
    ga = jnp.dot(sc, wm_s[:, 2 * D:3 * D], preferred_element_type=F32)[0:1, :]
    mod_r = jnp.dot(sc, wm_s[:, 3 * D:6 * D], preferred_element_type=F32)
    sb, cb1, gb = mod_r[0:1, 0:D], 1.0 + mod_r[0:1, D:2 * D], mod_r[0:1, 2 * D:3 * D]

    def resid(r, ga_):
        return x_s[r, :].astype(F32) + ga_ * acc_s[r, :]

    def h2_blocks(r0, n, ga_, sb_, cb1_):
        r = pl.ds(pl.multiple_of(r0, n), n)
        return _to_blocks((_ln(resid(r, ga_)) * cb1_ + sb_).astype(BF))

    for ch in range(2):
        for b, blk in enumerate(h2_blocks(ch * (TM // 2), TM // 2, ga, sb, cb1)):
            h_s[b, ch * (TM // 4):(ch + 1) * (TM // 4), :] = blk
    mod_s[2:3, :] = ga
    mod_s[3:4, :] = sb
    mod_s[4:5, :] = cb1
    mod_s[5:6, :] = gb

    def ffn_body(i, carry):
        r = pl.ds(pl.multiple_of(i * TM, TM), TM)
        h2 = load_h(pl.ds(pl.multiple_of(i * (TM // 2), TM // 2), TM // 2))
        inext = lax.rem(i + 1, NTM)

        rc = TM // len(DEP)
        zs = []
        for ch in range(len(DEP)):
            blks = h2_blocks(inext * TM + ch * rc, rc, mod_s[2:3, :], mod_s[3:4, :], mod_s[4:5, :])
            z = None
            for rr in range(rc // 16):
                for b in range(NB):
                    piece = blks[b][rr * 8:(rr + 1) * 8, :]
                    z = piece if z is None else (z | piece)
            zs.append(z & zero_s[...])
            for b in range(NB):
                hn_s[b, ch * rc // 2:(ch + 1) * rc // 2, :] = blks[b]

        def tied(w_ref, which):
            parts, pos = [], 0
            for ch, (wh, cb) in enumerate(DEP):
                if wh != which:
                    continue
                c0 = cb * 128
                if c0 > pos:
                    parts.append(w_ref[:, pos:c0])
                blk = pltpu.bitcast(w_ref[:, c0:c0 + 128], U32) | jnp.tile(zs[ch], (D // 16, 1))
                parts.append(pltpu.bitcast(blk, BF))
                pos = c0 + 128
            if pos < F:
                parts.append(w_ref[:, pos:])
            return jnp.concatenate(parts, axis=1)

        g = jnp.dot(h2, tied(wg_s, 'g'), preferred_element_type=F32)
        u = jnp.dot(h2, tied(wu_s, 'u'), preferred_element_type=F32)
        a = (_gelu(g) * u).astype(BF)
        y = jnp.dot(a, wd_s[...], preferred_element_type=F32)
        res = (resid(r, mod_s[2:3, :]) + mod_s[5:6, :] * y).astype(BF)
        pr = TM // OSP
        for pz in range(OSP):
            rp = pl.ds(pl.multiple_of(i * TM + pz * pr, pr), pr)
            o_s[rp, :] = res[pz * pr:(pz + 1) * pr]
            pltpu.make_async_copy(o_s.at[rp, :], o_hbm.at[0, rp, :], o_sem.at[0]).start()
        r2n = pl.ds(pl.multiple_of(inext * (TM // 2), TM // 2), TM // 2)
        for b in range(NB):
            h_s[b, r2n, :] = hn_s[b]
        return carry

    lax.fori_loop(0, NTM, ffn_body, 0)
    k_copy(0, (H - 1) % 2).wait()
    pltpu.make_async_copy(o_s, o_hbm.at[0], o_sem.at[0]).wait()


@jax.jit
def pallas_adaLN_cond__mha_block_cached__geglu_ffn__prompt_kernel(
    A_x: jax.Array,
    A_k_cache: jax.Array,
    A_v_cache: jax.Array,
    A_wq: jax.Array,
    A_wo: jax.Array,
    B_x: jax.Array,
    B_w_gate: jax.Array,
    B_w_up: jax.Array,
    B_w_down: jax.Array,
    c: jax.Array,
    w_mod: jax.Array,
):
    del B_x
    any_spec = pl.BlockSpec(memory_space=pl.ANY)
    return pl.pallas_call(
        _kernel,
        in_specs=[any_spec] * 10,
        out_specs=any_spec,
        out_shape=jax.ShapeDtypeStruct((1, S, D), A_x.dtype),
        scratch_shapes=[
            pltpu.VMEM((S, D), BF),
            pltpu.VMEM((2, SK, DH), BF),
            pltpu.VMEM((2, SK, DH), BF),
            pltpu.VMEM((H + 2, D, DH), BF),
            pltpu.VMEM((H + 2, NB, DH, 128), BF),
            pltpu.VMEM((D, F), BF),
            pltpu.VMEM((D, F), BF),
            pltpu.VMEM((F, D), BF),
            pltpu.VMEM((1, D), BF),
            pltpu.VMEM((D, 6 * D), BF),
            pltpu.VMEM((NB, S // 2, 128), U32),
            pltpu.VMEM((S, D), F32),
            pltpu.VMEM((8, D), F32),
            pltpu.VMEM((S, D), BF),
            pltpu.VMEM((max(RS), DH), BF),
            pltpu.VMEM((OPLAG, max(RS), DH), BF),
            pltpu.VMEM((NB, TM // 2, 128), U32),
            pltpu.VMEM((8, 128), U32),
            pltpu.SemaphoreType.DMA((4,)),
            pltpu.SemaphoreType.DMA((3,)),
            pltpu.SemaphoreType.DMA((9,)),
            pltpu.SemaphoreType.DMA((1,)),
        ],
        compiler_params=pltpu.CompilerParams(
            vmem_limit_bytes=100 * 1024 * 1024,
            disable_bounds_checks=True,
            disable_semaphore_checks=True,
        ),
    )(A_x, A_k_cache, A_v_cache, A_wq, A_wo, B_w_gate, B_w_up, B_w_down, c, w_mod)
```
